```python
import jax
import jax.numpy as jnp

def _softmax(x, axis=-1):
    return jax.nn.softmax(x, axis=axis)
def _gelu(x):
    return jax.nn.gelu(x, approximate=True)
def _silu(x):
    return jax.nn.silu(x)
def _sigmoid(x):
    return jax.nn.sigmoid(x)
def _layernorm(x, axis=-1, eps=1e-5):
    m = jnp.mean(x, axis=axis, keepdims=True)
    v = jnp.var(x, axis=axis, keepdims=True)
    return (x - m) / jnp.sqrt(v + eps)
def _scatter_add(tgt, idx, src, axis=0):
    return tgt.at[idx].add(src)
def _segment_sum(src, seg, n):
    return jax.ops.segment_sum(src, seg, n)
class _Rng:
    def __init__(self, key):
        self._k = key
    def _next(self):
        self._k, sub = jax.random.split(self._k)
        return sub
    def normal(self, shape):
        return jax.random.normal(self._next(), shape, dtype=jnp.bfloat16)
    def randint(self, lo, hi, shape):
        return jax.random.randint(self._next(), shape, lo, hi, dtype=jnp.int32)
    def uniform(self, shape, lo=0.0, hi=1.0):
        return jax.random.uniform(self._next(), shape, jnp.bfloat16, lo, hi)
    def permutation(self, n):
        return jax.random.permutation(self._next(), n)


kernel_name = 'standalone__modern_conv_block_slak__vision'

def setup_inputs():
    _rng = _Rng(jax.random.key(int.from_bytes(__import__("os").urandom(4), "little")))
    _w = (lambda a: (lambda t: t.astype(jnp.bfloat16) if jnp.issubdtype(t.dtype, jnp.floating) else t)(jnp.asarray(a)))
    H = W = 384
    C = 384
    K = 1
    return {
        "x": _w((lambda *s: _rng.normal(s) * 0.05)(1, H, W, C)),
        "dw": _w((lambda *s: _rng.normal(s) * 0.05)(K, K, C)),
        "w1": _w((lambda *s: _rng.normal(s) * 0.05)(C, 4 * C)),
        "w2": _w((lambda *s: _rng.normal(s) * 0.05)(4 * C, C)),
        "grn_g": _w((lambda *s: _rng.normal(s) * 0.05)(4 * C)),
        "grn_b": _w((lambda *s: _rng.normal(s) * 0.05)(4 * C)),
    }

def reference(x, dw, w1, w2, grn_g, grn_b):
    B, H, W, C = x.shape
    K = dw.shape[0]
    pad = K // 2
    xp = jnp.pad(x, ((0,0),(pad,pad),(pad,pad),(0,0)))
    out = jnp.zeros_like(x)
    for i in range(K):
        for j in range(K):
            out = out + xp[:, i:i+H, j:j+W, :] * dw[i, j][None, None, None, :]
    h = _layernorm(out, axis=-1)
    h = _gelu(h @ w1)
    gx = jnp.sqrt((h * h).sum(axis=(1, 2), keepdims=True) + 1e-6)
    nx = gx / (gx.mean(axis=-1, keepdims=True) + 1e-6)
    h = grn_g[None, None, None, :] * (h * nx) + grn_b[None, None, None, :] + h
    return x + h @ w2
```

```python
import functools
import numpy as np
import jax
import jax.numpy as jnp
import jax.experimental.pallas as pl
import jax.experimental.pallas.tpu as pltpu

TM = 2048
SUB = 256
RES = 0
VMEM_MB = 120

_C0 = float(np.sqrt(2.0 / np.pi))
_C1 = 0.044715 * _C0
_A = _C1 ** (1.0 / 3.0)
_K0 = _C0 / _A
_HS = 0.5 / _A


def _body(x_ref, dw_ref, w1_ref, w2_ref, g_ref, b_ref, o_ref, h_hbm,
          hbuf, ssq, w2s, bias, sems, *, tm, sub, nt):
    p = pl.program_id(0)
    i = pl.program_id(1)
    slot = i % 2

    def h_out(t, s):
        return pltpu.make_async_copy(hbuf.at[s], h_hbm.at[pl.ds(t * tm, tm)], sems.at[s])

    def h_in(t, s):
        return pltpu.make_async_copy(h_hbm.at[pl.ds(t * tm, tm)], hbuf.at[s], sems.at[s])

    @pl.when(p == 0)
    def _phase1():
        @pl.when(i == 0)
        def _():
            ssq[...] = jnp.zeros_like(ssq)

        @pl.when(i >= 2)
        def _():
            h_out(i - 2, slot).wait()

        dw = dw_ref[...].astype(jnp.float32)
        acc = ssq[...]
        for j in range(tm // sub):
            rows = pl.ds(j * sub, sub)
            o = x_ref[rows, :].astype(jnp.float32) * dw
            m = jnp.mean(o, axis=-1, keepdims=True)
            d = o - m
            v = jnp.mean(d * d, axis=-1, keepdims=True)
            ln = (d * (_A * jax.lax.rsqrt(v + 1e-5))).astype(jnp.bfloat16)
            z = jnp.dot(ln, w1_ref[...], preferred_element_type=jnp.float32)
            th = jnp.tanh(z * (z * z + _K0))
            h = z * th + z
            acc = acc + (h * h).reshape(sub // 8, 8, h.shape[-1]).sum(axis=0)
            hbuf[slot, rows, :] = h.astype(jnp.bfloat16)
        ssq[...] = acc
        h_out(i, slot).start()

        @pl.when(i == nt - 1)
        def _():
            h_out(i - 1, 1 - slot).wait()
            h_out(i, slot).wait()
            h_in(0, 0).start()
            tot = jnp.sum(ssq[...], axis=0, keepdims=True) * (_HS * _HS)
            gx = jnp.sqrt(tot + 1e-6)
            nx = gx / (jnp.mean(gx, axis=-1, keepdims=True) + 1e-6)
            s = (g_ref[...].astype(jnp.float32) * nx + 1.0) * _HS
            n4 = s.shape[-1]
            for c in range(n4 // 128):
                sc = jnp.broadcast_to(s[:, c * 128:(c + 1) * 128], (128, 128)).T
                wv = w2_ref[pl.ds(c * 128, 128), :].astype(jnp.float32)
                w2s[pl.ds(c * 128, 128), :] = (wv * jnp.concatenate([sc] * (wv.shape[-1] // 128), axis=1)).astype(jnp.bfloat16)
            bb = jnp.broadcast_to(b_ref[...], (8, n4))
            bias[...] = jnp.dot(bb, w2_ref[...], preferred_element_type=jnp.float32)

    @pl.when(p == 1)
    def _phase2():
        @pl.when(i + 1 < nt)
        def _():
            h_in(i + 1, 1 - slot).start()
        h_in(i, slot).wait()
        bv = bias[0:1, :]
        for j in range(tm // sub):
            rows = pl.ds(j * sub, sub)
            y = jnp.dot(hbuf[slot, rows, :], w2s[...], preferred_element_type=jnp.float32)
            o_ref[rows, :] = (x_ref[rows, :].astype(jnp.float32) + bv + y).astype(o_ref.dtype)


@jax.jit
def pallas_standalone__modern_conv_block_slak__vision_kernel(x, dw, w1, w2, grn_g, grn_b):
    B, H, W, C = x.shape
    assert B == 1 and dw.shape[0] == 1 and dw.shape[1] == 1
    n = H * W
    c4 = w1.shape[1]
    tm, sub = TM, SUB
    nt = n // tm
    x2 = x.reshape(n, C)
    const = lambda p, i: (0, 0)
    out, _ = pl.pallas_call(
        functools.partial(_body, tm=tm, sub=sub, nt=nt),
        grid=(2, nt),
        in_specs=[
            pl.BlockSpec((tm, C), lambda p, i: (i, 0)),
            pl.BlockSpec((1, C), const),
            pl.BlockSpec((C, c4), const),
            pl.BlockSpec((c4, C), const),
            pl.BlockSpec((1, c4), const),
            pl.BlockSpec((1, c4), const),
        ],
        out_specs=[
            pl.BlockSpec((tm, C), lambda p, i: (i * p, 0)),
            pl.BlockSpec(memory_space=pl.ANY),
        ],
        out_shape=[
            jax.ShapeDtypeStruct((n, C), x.dtype),
            jax.ShapeDtypeStruct((n, c4), jnp.bfloat16),
        ],
        scratch_shapes=[
            pltpu.VMEM((2, tm, c4), jnp.bfloat16),
            pltpu.VMEM((8, c4), jnp.float32),
            pltpu.VMEM((c4, C), jnp.bfloat16),
            pltpu.VMEM((8, C), jnp.float32),
            pltpu.SemaphoreType.DMA((2,)),
        ],
        compiler_params=pltpu.CompilerParams(
            dimension_semantics=("arbitrary", "arbitrary"),
            vmem_limit_bytes=VMEM_MB * 1024 * 1024,
        ),
    )(x2, dw.reshape(1, C), w1, w2, grn_g.reshape(1, c4), grn_b.reshape(1, c4))
    return out.reshape(B, H, W, C)
```

```python
import functools
import numpy as np
import jax
import jax.numpy as jnp
from jax.experimental import pallas as pl
from jax.experimental.pallas import tpu as pltpu

TM = 1536
R1 = 64
R2 = 64
NRES = 68
NSTG = 3
ORDER = (14, 13, 7, 11, 15, 8, 12, 10, 1, 9, 3, 6, 5, 2, 4)
OFFS = (0, 1, 7, 8)
LNT = (0, 1, 3, 5, 7, 9, 11, 13)
ORDER2 = (14, 13, 7, 11, 15, 8, 12, 10, 1, 9, 3, 6, 5, 2, 4)
VMEM_BYTES = 128 * 1024 * 1024
FLAGS = None
GA = 16
DMA1 = True
DMA2 = True
P2 = True
PIN2 = True
FSPAN = 12

_C0 = float(np.sqrt(2.0 / np.pi))
_C1 = 0.044715 * _C0
_A = _C1 ** (1.0 / 3.0)
_K0 = _C0 / _A
_HS = 0.5 / _A

S1 = dict(m=2, k=3, n=3,
     us=[(0, 1, 3, -1), (6, 1, 5, -1), (1, 1, 2, -1), (1, 1, 4, -1), (8, 1, 4, -1), (0, 1, 1, 1), (7, 1, 2, 1), (0, 1, 4, 1), (6, -1, 13, 1), (0, 1, 7, -1), (8, 1, 15, 1)],
     un=[5, 16, 15, 2, 13, 9, 4, 6, 11, 10, 0, 8, 12, 14, 7],
     ws=[(0, 1, 2, -1), (0, 1, 1, 1), (0, 1, 3, 1), (6, 1, 3, 1), (9, 1, 5, -1), (1, 1, 8, 1), (10, 1, 4, 1), (11, 1, 4, 1), (13, 1, 5, -1), (1, 1, 12, 1)],
     wn=[5, 12, 10, 2, 11, 7, 13, 3, 1, 14, 8, 15, 6, 4, 9],
     v=[[0, 0, -1, 0, 0, 0, 0, 0, 1], [0, 0, 0, 0, 0, 0, 0, 1, 0], [0, 0, -1, 0, 0, 0, 0, -1, 0], [0, 0, 0, 0, 0, 1, 1, 0, 1], [0, 1, 0, 1, -1, 0, 0, -1, 0], [0, 0, 0, 1, 0, 0, 0, 0, 0], [0, -1, 0, 0, 1, 1, 0, 1, 0], [-1, 0, 0, 0, 0, 0, 1, 0, 0], [0, 0, 0, -1, 1, 0, 0, 1, 0], [0, 0, 0, 0, 0, 1, 0, 0, 0], [1, -1, 1, -1, 1, 0, 0, 1, 0], [0, 0, 0, 0, 0, -1, 0, -1, 0], [0, 0, 0, 0, 0, 0, 1, 0, 0], [0, 1, 0, 0, 0, 0, 0, -1, 0], [0, 0, -1, 0, 0, 0, -1, 0, 0]])


def _addsub(a, sa, b, sb):
    if sa == sb:
        return a + b, sa
    return (a - b, 1) if sa > 0 else (b - a, 1)


def _forms(vals, steps):
    nodes = [(v, 1) for v in vals]
    for a, sa, b, sb in steps:
        nodes.append(_addsub(nodes[a][0], sa * nodes[a][1], nodes[b][0], sb * nodes[b][1]))
    return nodes


def _combine(prods, steps, wn, nout):
    adj = [[] for _ in range(nout + len(steps))]
    for r, node in enumerate(wn):
        adj[node].append(prods[r])

    def total(lst):
        acc = lst[0]
        for v in lst[1:]:
            acc = _addsub(acc[0], acc[1], v[0], v[1])
        return acc

    for t in reversed(range(len(steps))):
        a, sa, b, sb = steps[t]
        v, s = total(adj[nout + t])
        adj[a].append((v, s * sa))
        adj[b].append((v, s * sb))
    return [total(adj[o]) for o in range(nout)]


def _weight_forms(block, v):
    acc = None
    for idx, c in enumerate(v):
        if c:
            t = block(idx)
            acc = (t if c > 0 else -t) if acc is None else (acc + t if c > 0 else acc - t)
    return acc


def _pk(v):
    return pltpu.bitcast(v.astype(jnp.bfloat16), jnp.uint32)


def _unpk(w):
    return pltpu.bitcast(w, jnp.bfloat16)


def _zip(v):
    g = v.shape[0] // 16
    half = [jnp.concatenate([v[16 * i + 8 * e:16 * i + 8 * e + 8] for i in range(g)], axis=0) for e in range(2)]
    return pltpu.pack_elementwise(half, packed_dtype=jnp.bfloat16)


def _unzip(w):
    half = [pltpu.unpack_elementwise(w, index=e, packed_dtype=jnp.bfloat16, unpacked_dtype=jnp.float32)
            for e in range(2)]
    return jnp.concatenate([half[e][8 * i:8 * i + 8] for i in range(w.shape[0] // 8) for e in range(2)], axis=0)


def _body(tab_ref, x_ref, dw_ref, w1_ref, w2_ref, g_ref, b_ref, o_ref, h_hbm,
          hbuf, ssq, vw, fm, fm2, tot, lns, bias, sems, *, tm, nt):
    s = pl.program_id(0)
    f32, bf16 = jnp.float32, jnp.bfloat16
    C, C4 = w1_ref.shape
    nb = C4 // 3
    nunit = (tm // R1) * (C4 // 128)
    nstr = nunit - NRES

    def ring(t):
        return hbuf.at[pl.ds(nt * NRES + (t % NSTG) * nstr, nstr)]

    def resident(t):
        return hbuf.at[pl.ds(t * NRES, NRES)]

    def unit(views, blk, col):
        u = blk * (C4 // 128) + col // 128
        return views[0].at[u] if u < nstr else views[1].at[u - nstr]

    def h_out(t):
        return pltpu.make_async_copy(ring(t), h_hbm.at[t], sems.at[t % NSTG])

    def h_in(t):
        return pltpu.make_async_copy(h_hbm.at[t], ring(t), sems.at[t % NSTG])

    usgn = [sg for _, sg in _forms([0.0] * 6, S1["us"])]
    contrib = {n: [] for n in range(16)}
    for t, (a, sa, b, sb) in enumerate(S1["ws"]):
        contrib[a].append((6 + t, sa))
        contrib[b].append((6 + t, sb))
    prod_of = {n: r for r, n in enumerate(S1["wn"])}
    dep1 = [False] * 3 + [True] * 3
    for a, _, b, _ in S1["us"]:
        dep1.append(dep1[a] or dep1[b])

    def total_signs(order):
        sg = {}
        for n in order:
            acc = usgn[S1["un"][prod_of[n]]]
            for src, c in contrib[n]:
                acc = _addsub(0.0, acc, 0.0, c * sg[src])[1]
            sg[n] = acc
        return sg

    def absorb(order, q, p, tref, emit):
        tsgn = total_signs(order)
        n = order[q]
        acc = (p, usgn[S1["un"][prod_of[n]]])
        for src, c in contrib[n]:
            acc = _addsub(acc[0], acc[1], tref[src - 6], c * tsgn[src])
        if n < 6:
            emit(n, *acc)
            return
        keep = any(src == n for m in order[q + 1:] for src, _ in contrib[m])
        for o in range(6):
            if o not in prod_of and any(src == n for src, _ in contrib[o]):
                if all(src in order[:q + 1] for src, _ in contrib[o]):
                    z = (acc[0], acc[1] * [c for src, c in contrib[o] if src == n][0])
                    for src, c in contrib[o]:
                        if src != n:
                            z = _addsub(z[0], z[1], tref[src - 6], c * tsgn[src])
                    emit(o, *z)
                else:
                    keep = True
        if keep:
            tref[n - 6] = acc[0]

    def phase1(cur, prv, pad, drain):
        R = R1
        nsub = tm // (2 * R)
        dw = dw_ref[...].astype(f32)

        def ln_piece(j, gg):
            g, ib = divmod(gg, 2)
            o = x_ref[pl.ds((2 * j + ib) * R + g * GA, GA), :].astype(f32) * dw
            d = o - jnp.sum(o, axis=-1, keepdims=True) * (1.0 / C)
            v = jnp.sum(d * d, axis=-1, keepdims=True) * (1.0 / (C * _A * _A)) + 1e-5 / (_A * _A)
            ln = d * jax.lax.rsqrt(v)
            blk = [ln[:, k * 128:(k + 1) * 128] for k in range(3)]
            if ib == 0:
                lns[g] = ln
                nodes = _forms(blk + blk, S1["us"])
                f = nodes[8][0]
            else:
                nodes = _forms([lns[g, :, pl.ds(k * 128, 128)] for k in range(3)] + blk, S1["us"])
                f = nodes[14][0]
            pad[NRES - 1, pl.ds(0, 8), :] = _zip(f)
            for r, u in enumerate(S1["un"]):
                if dep1[u] == (ib == 1):
                    fm[j % 3, r, pl.ds(g * 8, 8), :] = _zip(nodes[u][0])

        def step(j, q, c):
            def emit(o, z, sg):
                ib, jb = divmod(o, 3)
                col = jb * nb + c * 128
                th = jnp.tanh(z * (z * z + _K0))
                h = z * th + z if sg > 0 else z * th - z
                ssq[:, pl.ds(col, 128)] += (h * h).reshape(R // 8, 8, 128).sum(axis=0)
                unit(cur if j >= 0 else prv, 2 * (j % nsub) + ib, col)[...] = _zip(h)

            r = prod_of[ORDER[q]]
            p = jnp.dot(_unpk(fm[j % 3, r]), _unpk(vw[r, c]), preferred_element_type=f32)
            absorb(ORDER, q, p, tot.at[c], emit)

        for t in range(15 + max(OFFS) if drain else 15 * nsub):
            for c in range(4):
                jj, q = divmod(t - OFFS[c], 15)
                if not (drain and jj > 0):
                    step(jj - 1, q, c)
            if not drain:
                j, q = divmod(t, 15)
                for gg, tq in enumerate(LNT):
                    if tq == q:
                        ln_piece(j, gg)

    @pl.when(s == 0)
    def _init():
        ssq[...] = jnp.zeros_like(ssq)
        fm[...] = jnp.zeros_like(fm)
        tot[...] = jnp.zeros_like(tot)
        for c in range(4):
            blk = lambda idx: w1_ref[pl.ds((idx // 3) * 128, 128), pl.ds((idx % 3) * nb + c * 128, 128)].astype(f32)
            for r in range(15):
                vw[r, c] = _pk(_weight_forms(blk, S1["v"][r]))

    @pl.when(s < nt)
    def _phase1():
        @pl.when(jnp.logical_and(s >= NSTG, DMA1))
        def _():
            h_out(s - NSTG).wait()

        slot = tab_ref[0, s]
        phase1((hbuf.at[pl.ds(slot, nstr)], resident(s)), (None, resident(jnp.maximum(s - 1, 0))),
               resident(tab_ref[1, s]), False)

        @pl.when(jnp.logical_and(s < nt - NSTG, DMA1))
        def _():
            h_out(s).start()

    @pl.when(s == nt)
    def _finish_stats():
        phase1(None, (None, resident(nt - 1)), None, True)
        gx = jnp.sqrt(jnp.sum(ssq[...], axis=0, keepdims=True) * (_HS * _HS) + 1e-6)
        nx = gx / (jnp.mean(gx, axis=-1, keepdims=True) + 1e-6)
        sc = (g_ref[...].astype(f32) * nx + 1.0) * _HS
        for c in range(4):
            rows = [k * nb + c * 128 for k in range(3)]
            col = [jnp.broadcast_to(sc[:, r0:r0 + 128], (128, 128)).T for r0 in rows]
            blk = lambda idx: w2_ref[pl.ds(rows[idx // 3], 128), pl.ds((idx % 3) * 128, 128)].astype(f32) * col[idx // 3]
            for r in range(15):
                vw[r, c] = _pk(_weight_forms(blk, S1["v"][r]))
        bias[...] = jnp.dot(jnp.broadcast_to(b_ref[...], (8, C4)), w2_ref[...], preferred_element_type=f32)

    @pl.when(s > nt)
    def _phase2():
        t = 2 * nt - s

        @pl.when(jnp.logical_and(jnp.logical_and(t < nt - 1, t + 1 >= NSTG), DMA2))
        def _():
            h_in(t + 1 - NSTG).start()

        @pl.when(jnp.logical_and(t < nt - NSTG, DMA2))
        def _():
            h_in(t).wait()

        R = R2
        nsub = tm // (2 * R)
        cur = (hbuf.at[pl.ds(tab_ref[0, t], nstr)], resident(t))
        opaque = tab_ref[1, t] - t

        def form_piece(j, gc):
            g, c = divmod(gc, 4)
            blk = []
            for ib in range(2):
                for kb in range(3):
                    w = unit(cur, 2 * j + ib, kb * nb + c * 128)[pl.ds(8 * g, 8), :]
                    blk.append(_unpk(w).astype(f32))
            nodes = _forms(blk, S1["us"])
            if j > 0 and PIN2:
                tot[1 + opaque, 0, pl.ds(0, 8), :] = nodes[16][0][:8]
            for r, u in enumerate(S1["un"]):
                fm2[j % 2, r, c, pl.ds(8 * g, 8), :] = _zip(nodes[u][0])

        def step(j, q):
            def emit(o, y, sg):
                ib, jb = divmod(o, 3)
                rows, cols = pl.ds((2 * j + ib) * R, R), pl.ds(jb * 128, 128)
                base = _unzip(pltpu.bitcast(x_ref[rows, cols], jnp.uint32)) + bias[0:1, cols]
                o_ref[rows, cols] = _unpk(_zip(base + y if sg > 0 else base - y))

            r = prod_of[ORDER2[q]]
            p = [jnp.dot(_unpk(fm2[j % 2, r, c]), _unpk(vw[r, c]), preferred_element_type=f32) for c in range(4)]
            absorb(ORDER2, q, (p[0] + p[1]) + (p[2] + p[3]), tot.at[0], emit)

        npc = R // 4
        for gc in range(npc):
            form_piece(0, gc)
        for j in range(nsub):
            for q in range(15):
                step(j, q)
                if j + 1 < nsub:
                    for gc in range(npc):
                        if gc * FSPAN // npc == q:
                            form_piece(j + 1, gc)


@jax.jit
def pallas_standalone__modern_conv_block_slak__vision_kernel(x, dw, w1, w2, grn_g, grn_b):
    B, H, W, C = x.shape
    assert B == 1 and dw.shape[:2] == (1, 1) and C == 384 and w1.shape == (C, 4 * C)
    n = H * W
    c4 = 4 * C
    tm = TM
    nt = n // tm
    assert nt * tm == n and (tm // (2 * R1)) % 3 == 0 and R1 == R2
    nstr = (tm // R1) * (c4 // 128) - NRES
    assert NRES >= 4 * (c4 // 128)
    steps = np.arange(nt)
    table = np.stack([nt * NRES + (steps % NSTG) * nstr, steps]).astype(np.int32)
    whole = pl.BlockSpec(memory_space=pltpu.VMEM)
    scratch = [
        pltpu.VMEM((nt * NRES + NSTG * nstr, R1 // 2, 128), jnp.uint32),
        pltpu.VMEM((8, c4), jnp.float32),
        pltpu.VMEM((15, 4, 64, 128), jnp.uint32),
        pltpu.VMEM((3, 15, R1 // 2, 128), jnp.uint32),
        pltpu.VMEM((2, 15, 4, R2 // 2, 128), jnp.uint32),
        pltpu.VMEM((4, 10, R1, 128), jnp.float32),
        pltpu.VMEM((R1 // GA, GA, C), jnp.float32),
        pltpu.VMEM((8, C), jnp.float32),
        pltpu.SemaphoreType.DMA((NSTG,)),
    ]
    out, _ = pl.pallas_call(
        functools.partial(_body, tm=tm, nt=nt),
        grid_spec=pltpu.PrefetchScalarGridSpec(
            num_scalar_prefetch=1,
            grid=(2 * nt + 1 if P2 else nt + 1,),
            in_specs=[
                pl.BlockSpec((tm, C), lambda s, tab: (jnp.where(s < nt, s, jnp.minimum(2 * nt - s, nt - 1)), 0)),
                whole, whole, whole, whole, whole,
            ],
            out_specs=[
                pl.BlockSpec((tm, C), lambda s, tab: (jnp.minimum(2 * nt - s, nt - 1), 0)),
                pl.BlockSpec(memory_space=pl.ANY),
            ],
            scratch_shapes=scratch,
        ),
        out_shape=[
            jax.ShapeDtypeStruct((n, C), x.dtype),
            jax.ShapeDtypeStruct((nt - NSTG, nstr, R1 // 2, 128), jnp.uint32),
        ],
        compiler_params=pltpu.CompilerParams(
            dimension_semantics=("arbitrary",),
            vmem_limit_bytes=VMEM_BYTES,
            flags=FLAGS,
        ),
    )(table, x.reshape(n, C), dw.reshape(1, C), w1, w2, grn_g.reshape(1, c4), grn_b.reshape(1, c4))
    return out.reshape(B, H, W, C)
```

```python
import functools

import jax
import jax.numpy as jnp
import numpy as np
from jax.experimental import pallas as pl
from jax.experimental.pallas import tpu as pltpu

TM = 1536
TPS = 2
R = 64
NRES = 65
NSTG = 6
ORDER = (14, 13, 7, 11, 15, 8, 12, 10, 1, 9, 3, 6, 5, 2, 4)
OFFS = (0, 1, 7, 8)
LNT = (0, 1, 3, 5, 7, 9, 11, 13)
ORDER2 = (14, 13, 7, 11, 15, 8, 12, 10, 1, 9, 3, 6, 5, 2, 4)
REDO = (70, 45, 20)
FLAGS = None
HP = 1
XP = 0

_C0 = float(np.sqrt(2.0 / np.pi))
_C1 = 0.044715 * _C0
_A = _C1 ** (1.0 / 3.0)
_K0 = _C0 / _A
_HS = 0.5 / _A

_SCHEME = dict(
     us=[(0, 1, 3, -1), (6, 1, 5, -1), (1, 1, 2, -1), (1, 1, 4, -1), (8, 1, 4, -1), (0, 1, 1, 1), (7, 1, 2, 1), (0, 1, 4, 1), (6, -1, 13, 1), (0, 1, 7, -1), (8, 1, 15, 1)],
     un=[5, 16, 15, 2, 13, 9, 4, 6, 11, 10, 0, 8, 12, 14, 7],
     ws=[(0, 1, 2, -1), (0, 1, 1, 1), (0, 1, 3, 1), (6, 1, 3, 1), (9, 1, 5, -1), (1, 1, 8, 1), (10, 1, 4, 1), (11, 1, 4, 1), (13, 1, 5, -1), (1, 1, 12, 1)],
     wn=[5, 12, 10, 2, 11, 7, 13, 3, 1, 14, 8, 15, 6, 4, 9],
     v=[[0, 0, -1, 0, 0, 0, 0, 0, 1], [0, 0, 0, 0, 0, 0, 0, 1, 0], [0, 0, -1, 0, 0, 0, 0, -1, 0], [0, 0, 0, 0, 0, 1, 1, 0, 1], [0, 1, 0, 1, -1, 0, 0, -1, 0], [0, 0, 0, 1, 0, 0, 0, 0, 0], [0, -1, 0, 0, 1, 1, 0, 1, 0], [-1, 0, 0, 0, 0, 0, 1, 0, 0], [0, 0, 0, -1, 1, 0, 0, 1, 0], [0, 0, 0, 0, 0, 1, 0, 0, 0], [1, -1, 1, -1, 1, 0, 0, 1, 0], [0, 0, 0, 0, 0, -1, 0, -1, 0], [0, 0, 0, 0, 0, 0, 1, 0, 0], [0, 1, 0, 0, 0, 0, 0, -1, 0], [0, 0, -1, 0, 0, 0, -1, 0, 0]])


def _addsub(a, sa, b, sb):
    if sa == sb:
        return a + b, sa
    return (a - b, 1) if sa > 0 else (b - a, 1)


def _forms(vals, steps):
    nodes = [(v, 1) for v in vals]
    for a, sa, b, sb in steps:
        nodes.append(_addsub(nodes[a][0], sa * nodes[a][1], nodes[b][0], sb * nodes[b][1]))
    return nodes


def _combine(prods, steps, wn, nout):
    adj = [[] for _ in range(nout + len(steps))]
    for r, node in enumerate(wn):
        adj[node].append(prods[r])

    def total(lst):
        acc = lst[0]
        for v in lst[1:]:
            acc = _addsub(acc[0], acc[1], v[0], v[1])
        return acc

    for t in reversed(range(len(steps))):
        a, sa, b, sb = steps[t]
        v, s = total(adj[nout + t])
        adj[a].append((v, s * sa))
        adj[b].append((v, s * sb))
    return [total(adj[o]) for o in range(nout)]


def _weight_forms(block, v):
    acc = None
    for idx, c in enumerate(v):
        if c:
            t = block(idx)
            acc = (t if c > 0 else -t) if acc is None else (acc + t if c > 0 else acc - t)
    return acc


def _pk(v):
    return pltpu.bitcast(v.astype(jnp.bfloat16), jnp.uint32)


def _unpk(w):
    return pltpu.bitcast(w, jnp.bfloat16)


def _zip(v):
    g = v.shape[0] // 16
    half = [jnp.concatenate([v[16 * i + 8 * e:16 * i + 8 * e + 8] for i in range(g)], axis=0) for e in range(2)]
    return pltpu.pack_elementwise(half, packed_dtype=jnp.bfloat16)


def _unzip(w):
    half = [pltpu.unpack_elementwise(w, index=e, packed_dtype=jnp.bfloat16, unpacked_dtype=jnp.float32)
            for e in range(2)]
    return jnp.concatenate([half[e][8 * i:8 * i + 8] for i in range(w.shape[0] // 8) for e in range(2)], axis=0)


def _placement(nt, nstr):
    assert all(t + 4 < nt - NSTG and t + 1 not in REDO and t + 4 not in REDO for t in REDO)
    kept = [t for t in range(nt) if t not in REDO]
    sent = [t for t in kept if t < nt - NSTG]
    base = {t: k * NRES for k, t in enumerate(kept)}
    first = [base[t + 4] if t in REDO else base[t] for t in range(nt)]
    second = [base[t + 1] if t in REDO else base[t] for t in range(nt)]
    ring = [len(kept) * NRES + (t % NSTG) * nstr for t in range(nt)]
    hbm = [sent.index(t) if t in sent else (-2 if t in REDO else -1) for t in range(nt)]
    cuts = [0] + sorted(nt - 1 - t for t in REDO)
    cuts += [nt] * (nt - len(cuts))
    return np.array([ring, first, first, second, hbm, second, cuts], np.int32), len(kept), len(sent)


def _body(x_hbm, dw_ref, w1_hbm, w2_hbm, g_ref, b_ref, tab_ref, o_hbm, h_hbm,
          pool, hbuf, v1, v2, ssq, fm, tot, lns, bias, hsem, xsem, osem, wsem, *, nt):
    f32, bf16 = jnp.float32, jnp.bfloat16
    C, C4 = w1_hbm.shape
    nb = C4 // 3
    ncol = C4 // 128
    nsub = TM // (2 * R)
    nstr = 2 * nsub * ncol - NRES
    n1 = nt // TPS
    xside = (n1 - 1) % 2

    def ring(t):
        return hbuf.at[pl.ds(tab_ref[0, t], nstr)]

    def resident(row, t):
        return hbuf.at[pl.ds(tab_ref[row, t], NRES)]

    def unit(views, blk, col):
        u = blk * ncol + col // 128
        return views[0].at[u] if u < nstr else views[1].at[u - nstr]

    def if_streamed(t, fn):
        @pl.when(jnp.logical_and(t >= 0, tab_ref[4, jnp.maximum(t, 0)] >= 0))
        def _():
            fn()

    def h_out(t):
        return pltpu.make_async_copy(ring(t), h_hbm.at[tab_ref[4, t]], hsem.at[t % NSTG])

    def h_in(t):
        return pltpu.make_async_copy(h_hbm.at[tab_ref[4, t]], ring(t), hsem.at[t % NSTG])

    def x_step(i):
        return pltpu.make_async_copy(x_hbm.at[pl.ds(i * TPS, TPS)], pool.at[i % 2, pl.ds(2 - TPS, TPS)], xsem.at[i % 2])

    def x_tile(t):
        return pltpu.make_async_copy(x_hbm.at[t], pool.at[xside, t % 2], xsem.at[t % 2])

    def o_tile(t):
        return pltpu.make_async_copy(pool.at[1 - xside, t % 2], o_hbm.at[t], osem.at[t % 2])

    w1_copies = [pltpu.make_async_copy(w1_hbm.at[:, pl.ds(q * C, C)], pool.at[1, 0, pl.ds(q * C, C)], wsem.at[q])
                 for q in range(4)]
    w2_buf = pool.at[1 - xside, 0]
    w2_copy = pltpu.make_async_copy(w2_hbm, w2_buf, wsem.at[0])

    us, un, ws, wn = (_SCHEME[k] for k in ("us", "un", "ws", "wn"))
    usgn = [sg for _, sg in _forms([0.0] * 6, us)]
    ucoef = [_forms(list(np.eye(6, dtype=int)), us)[u][0] for u in un]
    assert all(cf.max() > 0 for cf in ucoef)
    contrib = {n: [] for n in range(6 + len(ws))}
    for t, (a, sa, b, sb) in enumerate(ws):
        contrib[a].append((6 + t, sa))
        contrib[b].append((6 + t, sb))
    prod_of = {n: r for r, n in enumerate(wn)}
    dep1 = [False] * 3 + [True] * 3
    for a, _, b, _ in us:
        dep1.append(dep1[a] or dep1[b])

    def absorb(order, q, p, tref, emit):
        tsgn = {}
        for n in order:
            tsgn[n] = usgn[un[prod_of[n]]]
            for src, c in contrib[n]:
                tsgn[n] = _addsub(0.0, tsgn[n], 0.0, c * tsgn[src])[1]
        n = order[q]
        acc = (p, usgn[un[prod_of[n]]])
        for src, c in contrib[n]:
            acc = _addsub(*acc, tref[src - 6], c * tsgn[src])
        if n < 6:
            emit(n, *acc)
            return
        keep = any(src == n for m in order[q + 1:] for src, _ in contrib[m])
        for o in range(6):
            if o not in prod_of and any(src == n for src, _ in contrib[o]):
                if all(src in order[:q + 1] for src, _ in contrib[o]):
                    z = (acc[0], acc[1] * [c for src, c in contrib[o] if src == n][0])
                    for src, c in contrib[o]:
                        if src != n:
                            z = _addsub(*z, tref[src - 6], c * tsgn[src])
                    emit(o, *z)
                else:
                    keep = True
        if keep:
            tref[n - 6] = acc[0]

    def expand(xs, views, prev, pin, first, last):
        dw = dw_ref[...].astype(f32)
        nj = len(views) * nsub

        def norm_piece(j, gg):
            g, ib = divmod(gg, 2)
            o = xs[j // nsub, pl.ds((2 * (j % nsub) + ib) * R + 16 * g, 16), :].astype(f32) * dw
            d = o - jnp.sum(o, axis=-1, keepdims=True) * (1.0 / C)
            v = jnp.sum(d * d, axis=-1, keepdims=True) * (1.0 / (C * _A * _A)) + 1e-5 / (_A * _A)
            ln = d * jax.lax.rsqrt(v)
            blk = [ln[:, k * 128:(k + 1) * 128] for k in range(3)]
            if ib == 0:
                lns[g] = ln
                nodes = _forms(blk + blk, us)
            else:
                nodes = _forms([lns[g, :, pl.ds(k * 128, 128)] for k in range(3)] + blk, us)
            pin[NRES - 1, pl.ds(0, 8), :] = _zip(nodes[14 if ib else 8][0])
            for r, u in enumerate(un):
                if dep1[u] == (ib == 1):
                    fm[j % 3, r, pl.ds(8 * g, 8), :] = _zip(nodes[u][0])

        def step(j, q, c):
            def emit(o, z, sg):
                ib, jb = divmod(o, 3)
                col = jb * nb + c * 128
                th = jnp.tanh(z * (z * z + _K0))
                h = z * th + z if sg > 0 else z * th - z
                ssq[:, pl.ds(col, 128)] += (h * h).reshape(R // 8, 8, 128).sum(axis=0)
                unit(views[j // nsub] if j >= 0 else (None, prev), 2 * (j % nsub) + ib, col)[...] = _zip(h)

            r = prod_of[ORDER[q]]
            p = jnp.dot(_unpk(fm[j % 3, r]), _unpk(v1[r, c]), preferred_element_type=f32)
            absorb(ORDER, q, p, tot.at[c], emit)

        for t in range(15 * nj if last is None else 15 * (last + 2) + max(OFFS)):
            for c in range(4):
                jj, q = divmod(t - OFFS[c], 15)
                if jj - 1 >= first and (last is None or jj - 1 <= last):
                    step(jj - 1, q, c)
            for gg, tq in enumerate(LNT):
                if tq == t % 15 and t // 15 < nj:
                    norm_piece(t // 15, gg)

    for cp in w1_copies:
        cp.start()
    x_step(0).start()
    ssq[...] = jnp.zeros_like(ssq)
    fm[...] = jnp.zeros_like(fm)
    tot[...] = jnp.zeros_like(tot)
    for cp in w1_copies:
        cp.wait()
    for c in range(4):
        def w1_block(idx):
            q, col = divmod((idx % 3) * nb + c * 128, C)
            return pool[1, 0, pl.ds(q * C + (idx // 3) * 128, 128), pl.ds(col, 128)].astype(f32)
        for r in range(15):
            v1[r, c] = _pk(_weight_forms(w1_block, _SCHEME["v"][r]))

    def phase1(i, carry):
        @pl.when(i + 1 < n1)
        def _():
            x_step(i + 1).start()

        @pl.when(i + 1 == n1)
        def _():
            w2_copy.start()

        tiles = [i * TPS + e for e in range(TPS)]
        for t in tiles:
            if_streamed(t - NSTG, lambda: h_out(t - NSTG).wait())
        x_step(i).wait()
        expand(pool.at[i % 2, pl.ds(2 - TPS, TPS)], [(ring(t), resident(1, t)) for t in tiles],
               resident(1, jnp.maximum(tiles[0] - 1, 0)), resident(2, tiles[-1]), -2, None)
        for t in tiles:
            if_streamed(t, lambda: h_out(t).start())
        return carry

    jax.lax.fori_loop(0, n1, phase1, 0)
    expand(None, [], resident(1, nt - 1), None, -2, -1)

    gx = jnp.sqrt(jnp.sum(ssq[...], axis=0, keepdims=True) * (_HS * _HS) + 1e-6)
    nx = gx / (jnp.mean(gx, axis=-1, keepdims=True) + 1e-6)
    scale = (g_ref[...].astype(f32).reshape(1, C4) * nx + 1.0) * _HS
    w2_copy.wait()
    for c in range(4):
        rows = [k * nb + c * 128 for k in range(3)]
        col = [jnp.broadcast_to(scale[:, r0:r0 + 128], (128, 128)).T for r0 in rows]

        def w2_block(idx):
            return w2_buf[pl.ds(rows[idx // 3], 128), pl.ds((idx % 3) * 128, 128)].astype(f32) * col[idx // 3]
        for r in range(15):
            v2[r, c] = _pk(_weight_forms(w2_block, _SCHEME["v"][r]))
    bias[...] = jnp.dot(jnp.broadcast_to(b_ref[...].astype(f32).reshape(1, C4), (8, C4)).astype(bf16), w2_buf[...], preferred_element_type=f32)

    def fetch(t):
        @pl.when(jnp.logical_and(t >= 1, t - 1 < nt - TPS))
        def _():
            x_tile(t - 1).start(priority=XP)

        if_streamed(jnp.where(t + 1 < nt, t + 1 - NSTG, -1), lambda: h_in(t + 1 - NSTG).start(priority=HP))

        @pl.when(t + 2 < nt)
        def _():
            o_tile(t + 2).wait()

        @pl.when(t < nt - TPS)
        def _():
            x_tile(t).wait()

        if_streamed(t, lambda: h_in(t).wait())

    def phase2(i, carry):
        t = nt - 1 - i

        @pl.when(tab_ref[4, t] != -2)
        def _():
            fetch(t)

        views = (ring(t), resident(3, t))
        xt, ot = pool.at[xside, t % 2], pool.at[1 - xside, t % 2]

        def operand(j, r, c):
            acc = None
            for idx in np.argsort(-ucoef[r], kind="stable"):
                if ucoef[r][idx]:
                    ib, kb = divmod(int(idx), 3)
                    v = _unpk(unit(views, 2 * j + ib, kb * nb + c * 128)[...]).astype(f32)
                    acc = v if acc is None else (acc + v if ucoef[r][idx] > 0 else acc - v)
            return _unpk(_zip(acc))

        def step(j, q):
            def emit(o, y, sg):
                ib, jb = divmod(o, 3)
                rows, cols = pl.ds((2 * j + ib) * R, R), pl.ds(jb * 128, 128)
                base = _unzip(pltpu.bitcast(xt[rows, cols], jnp.uint32)) + bias[0:1, cols]
                ot[rows, cols] = _unpk(_zip(base + y if sg > 0 else base - y))

            r = prod_of[ORDER2[q]]
            p = [jnp.dot(operand(j, r, c), _unpk(v2[r, c]), preferred_element_type=f32) for c in range(4)]
            absorb(ORDER2, q, (p[0] + p[1]) + (p[2] + p[3]), tot.at[0], emit)

        for j in range(nsub):
            for q in range(15):
                step(j, q)
        o_tile(t).start(priority=XP)
        return carry

    def segment(m, carry):
        @pl.when(m > 0)
        def _():
            t = nt - 1 - tab_ref[6, m]
            fetch(t)
            expand(pool.at[xside, pl.ds(t % 2, 1)], [(ring(t), resident(3, t))], None, resident(5, t), 0, nsub - 1)

        return jax.lax.fori_loop(tab_ref[6, m], tab_ref[6, m + 1], phase2, carry)

    jax.lax.fori_loop(0, len(REDO) + 1, segment, 0)
    o_tile(1).wait()
    o_tile(0).wait()


@jax.jit
def pallas_standalone__modern_conv_block_slak__vision_kernel(x, dw, w1, w2, grn_g, grn_b):
    B, H, W, C = x.shape
    c4 = 4 * C
    assert B == 1 and dw.shape == (1, 1, C) and C == 384 and w1.shape == (C, c4) and TM == c4
    nt = H * W // TM
    nsub = TM // (2 * R)
    nstr = 2 * nsub * (c4 // 128) - NRES
    assert nt * TM == H * W and nt % 2 == 0 and nsub % 3 == 0 and NRES >= 4 * (c4 // 128)
    table, nkept, nsent = _placement(nt, nstr)
    hbm = pl.BlockSpec(memory_space=pl.ANY)
    vmem = pl.BlockSpec(memory_space=pltpu.VMEM)
    out, _ = pl.pallas_call(
        functools.partial(_body, nt=nt),
        in_specs=[hbm, vmem, hbm, hbm, vmem, vmem, pl.BlockSpec(memory_space=pltpu.SMEM)],
        out_specs=[hbm, hbm],
        out_shape=[
            jax.ShapeDtypeStruct((nt, TM, C), x.dtype),
            jax.ShapeDtypeStruct((nsent, nstr, R // 2, 128), jnp.uint32),
        ],
        scratch_shapes=[
            pltpu.VMEM((2, 2, TM, C), x.dtype),
            pltpu.VMEM((nkept * NRES + NSTG * nstr, R // 2, 128), jnp.uint32),
            pltpu.VMEM((15, 4, 64, 128), jnp.uint32),
            pltpu.VMEM((15, 4, 64, 128), jnp.uint32),
            pltpu.VMEM((8, c4), jnp.float32),
            pltpu.VMEM((3, 15, R // 2, 128), jnp.uint32),
            pltpu.VMEM((4, 10, R, 128), jnp.float32),
            pltpu.VMEM((R // 16, 16, C), jnp.float32),
            pltpu.VMEM((8, C), jnp.float32),
            pltpu.SemaphoreType.DMA((NSTG,)),
            pltpu.SemaphoreType.DMA((2,)),
            pltpu.SemaphoreType.DMA((2,)),
            pltpu.SemaphoreType.DMA((4,)),
        ],
        compiler_params=pltpu.CompilerParams(vmem_limit_bytes=128 * 1024 * 1024, flags=FLAGS),
    )(x.reshape(nt, TM, C), dw.reshape(1, C), w1, w2, grn_g, grn_b, table)
    return out.reshape(B, H, W, C)
```

```python
import functools

import jax
import jax.numpy as jnp
import numpy as np
from jax.experimental import pallas as pl
from jax.experimental.pallas import tpu as pltpu

TM = 1536
TPS = 2
R = 64
NRES = 65
NSTG = 6
ORDER = (14, 13, 7, 11, 15, 8, 12, 10, 1, 9, 3, 6, 5, 2, 4)
OFFS = (0, 1, 7, 8)
LNT = (0, 1, 3, 5, 7, 9, 11, 13)
ORDER2 = (14, 13, 7, 11, 15, 8, 12, 10, 1, 9, 3, 6, 5, 2, 4)
REDO = (70, 45, 20)
FLAGS = None
NOBC = True
HP = 1

_C0 = float(np.sqrt(2.0 / np.pi))
_C1 = 0.044715 * _C0
_A = _C1 ** (1.0 / 3.0)
_K0 = _C0 / _A
_HS = 0.5 / _A

_SCHEME = dict(
     us=[(0, 1, 3, -1), (6, 1, 5, -1), (1, 1, 2, -1), (1, 1, 4, -1), (8, 1, 4, -1), (0, 1, 1, 1), (7, 1, 2, 1), (0, 1, 4, 1), (6, -1, 13, 1), (0, 1, 7, -1), (8, 1, 15, 1)],
     un=[5, 16, 15, 2, 13, 9, 4, 6, 11, 10, 0, 8, 12, 14, 7],
     ws=[(0, 1, 2, -1), (0, 1, 1, 1), (0, 1, 3, 1), (6, 1, 3, 1), (9, 1, 5, -1), (1, 1, 8, 1), (10, 1, 4, 1), (11, 1, 4, 1), (13, 1, 5, -1), (1, 1, 12, 1)],
     wn=[5, 12, 10, 2, 11, 7, 13, 3, 1, 14, 8, 15, 6, 4, 9],
     v=[[0, 0, -1, 0, 0, 0, 0, 0, 1], [0, 0, 0, 0, 0, 0, 0, 1, 0], [0, 0, -1, 0, 0, 0, 0, -1, 0], [0, 0, 0, 0, 0, 1, 1, 0, 1], [0, 1, 0, 1, -1, 0, 0, -1, 0], [0, 0, 0, 1, 0, 0, 0, 0, 0], [0, -1, 0, 0, 1, 1, 0, 1, 0], [-1, 0, 0, 0, 0, 0, 1, 0, 0], [0, 0, 0, -1, 1, 0, 0, 1, 0], [0, 0, 0, 0, 0, 1, 0, 0, 0], [1, -1, 1, -1, 1, 0, 0, 1, 0], [0, 0, 0, 0, 0, -1, 0, -1, 0], [0, 0, 0, 0, 0, 0, 1, 0, 0], [0, 1, 0, 0, 0, 0, 0, -1, 0], [0, 0, -1, 0, 0, 0, -1, 0, 0]])


def _addsub(a, sa, b, sb):
    if sa == sb:
        return a + b, sa
    return (a - b, 1) if sa > 0 else (b - a, 1)


def _forms(vals, steps):
    nodes = [(v, 1) for v in vals]
    for a, sa, b, sb in steps:
        nodes.append(_addsub(nodes[a][0], sa * nodes[a][1], nodes[b][0], sb * nodes[b][1]))
    return nodes


def _combine(prods, steps, wn, nout):
    adj = [[] for _ in range(nout + len(steps))]
    for r, node in enumerate(wn):
        adj[node].append(prods[r])

    def total(lst):
        acc = lst[0]
        for v in lst[1:]:
            acc = _addsub(acc[0], acc[1], v[0], v[1])
        return acc

    for t in reversed(range(len(steps))):
        a, sa, b, sb = steps[t]
        v, s = total(adj[nout + t])
        adj[a].append((v, s * sa))
        adj[b].append((v, s * sb))
    return [total(adj[o]) for o in range(nout)]


def _weight_forms(block, v):
    acc = None
    for idx, c in enumerate(v):
        if c:
            t = block(idx)
            acc = (t if c > 0 else -t) if acc is None else (acc + t if c > 0 else acc - t)
    return acc


def _pk(v):
    return pltpu.bitcast(v.astype(jnp.bfloat16), jnp.uint32)


def _unpk(w):
    return pltpu.bitcast(w, jnp.bfloat16)


def _zip(v):
    g = v.shape[0] // 16
    half = [jnp.concatenate([v[16 * i + 8 * e:16 * i + 8 * e + 8] for i in range(g)], axis=0) for e in range(2)]
    return pltpu.pack_elementwise(half, packed_dtype=jnp.bfloat16)


def _unzip(w):
    half = [pltpu.unpack_elementwise(w, index=e, packed_dtype=jnp.bfloat16, unpacked_dtype=jnp.float32)
            for e in range(2)]
    return jnp.concatenate([half[e][8 * i:8 * i + 8] for i in range(w.shape[0] // 8) for e in range(2)], axis=0)


def _placement(nt, nstr):
    assert all(t + 4 < nt - NSTG and t + 1 not in REDO and t + 4 not in REDO for t in REDO)
    kept = [t for t in range(nt) if t not in REDO]
    sent = [t for t in kept if t < nt - NSTG]
    base = {t: k * NRES for k, t in enumerate(kept)}
    first = [base[t + 4] if t in REDO else base[t] for t in range(nt)]
    second = [base[t + 1] if t in REDO else base[t] for t in range(nt)]
    ring = [len(kept) * NRES + (t % NSTG) * nstr for t in range(nt)]
    hbm = [sent.index(t) if t in sent else (-2 if t in REDO else -1) for t in range(nt)]
    cuts = [0] + sorted(nt - 1 - t for t in REDO)
    cuts += [nt] * (nt - len(cuts))
    return np.array([ring, first, first, second, hbm, second, cuts, [t % NSTG for t in range(nt)]], np.int32), len(kept), len(sent)


def _body(x_hbm, dw_ref, w1_hbm, w2_hbm, g_ref, b_ref, tab_ref, o_hbm, h_hbm,
          pool, hbuf, v1, v2, ssq, fm, tot, lns, bias, hsem, xsem, osem, wsem, *, nt):
    f32, bf16 = jnp.float32, jnp.bfloat16
    C, C4 = w1_hbm.shape
    nb = C4 // 3
    ncol = C4 // 128
    nsub = TM // (2 * R)
    nstr = 2 * nsub * ncol - NRES
    n1 = nt // TPS
    xside = (n1 - 1) % 2

    def ring(t):
        return hbuf.at[pl.ds(tab_ref[0, t], nstr)]

    def resident(row, t):
        return hbuf.at[pl.ds(tab_ref[row, t], NRES)]

    def unit(views, blk, col):
        u = blk * ncol + col // 128
        return views[0].at[u] if u < nstr else views[1].at[u - nstr]

    def if_streamed(t, fn):
        @pl.when(jnp.logical_and(t >= 0, tab_ref[4, jnp.maximum(t, 0)] >= 0))
        def _():
            fn()

    def h_out(t):
        return pltpu.make_async_copy(ring(t), h_hbm.at[tab_ref[4, t]], hsem.at[tab_ref[7, t]])

    def h_in(t):
        return pltpu.make_async_copy(h_hbm.at[tab_ref[4, t]], ring(t), hsem.at[tab_ref[7, t]])

    def x_step(i):
        return pltpu.make_async_copy(x_hbm.at[pl.ds(i * TPS, TPS)], pool.at[i & 1, pl.ds(2 - TPS, TPS)], xsem.at[i & 1])

    def x_tile(t):
        return pltpu.make_async_copy(x_hbm.at[t], pool.at[xside, t & 1], xsem.at[t & 1])

    def o_tile(t):
        return pltpu.make_async_copy(pool.at[1 - xside, t & 1], o_hbm.at[t], osem.at[t & 1])

    w1_copies = [pltpu.make_async_copy(w1_hbm.at[:, pl.ds(q * C, C)], pool.at[1, 0, pl.ds(q * C, C)], wsem.at[q])
                 for q in range(4)]
    w2_buf = pool.at[1 - xside, 0]
    w2_copy = pltpu.make_async_copy(w2_hbm, w2_buf, wsem.at[0])

    us, un, ws, wn = (_SCHEME[k] for k in ("us", "un", "ws", "wn"))
    usgn = [sg for _, sg in _forms([0.0] * 6, us)]
    ucoef = [_forms(list(np.eye(6, dtype=int)), us)[u][0] for u in un]
    assert all(cf.max() > 0 for cf in ucoef)
    contrib = {n: [] for n in range(6 + len(ws))}
    for t, (a, sa, b, sb) in enumerate(ws):
        contrib[a].append((6 + t, sa))
        contrib[b].append((6 + t, sb))
    prod_of = {n: r for r, n in enumerate(wn)}
    dep1 = [False] * 3 + [True] * 3
    for a, _, b, _ in us:
        dep1.append(dep1[a] or dep1[b])

    def absorb(order, q, p, tref, emit):
        tsgn = {}
        for n in order:
            tsgn[n] = usgn[un[prod_of[n]]]
            for src, c in contrib[n]:
                tsgn[n] = _addsub(0.0, tsgn[n], 0.0, c * tsgn[src])[1]
        n = order[q]
        acc = (p, usgn[un[prod_of[n]]])
        for src, c in contrib[n]:
            acc = _addsub(*acc, tref[src - 6], c * tsgn[src])
        if n < 6:
            emit(n, *acc)
            return
        keep = any(src == n for m in order[q + 1:] for src, _ in contrib[m])
        for o in range(6):
            if o not in prod_of and any(src == n for src, _ in contrib[o]):
                if all(src in order[:q + 1] for src, _ in contrib[o]):
                    z = (acc[0], acc[1] * [c for src, c in contrib[o] if src == n][0])
                    for src, c in contrib[o]:
                        if src != n:
                            z = _addsub(*z, tref[src - 6], c * tsgn[src])
                    emit(o, *z)
                else:
                    keep = True
        if keep:
            tref[n - 6] = acc[0]

    def expand(xs, views, prev, pin, first, last):
        dw = dw_ref[...].astype(f32)
        nj = len(views) * nsub

        def norm_piece(j, gg):
            g, ib = divmod(gg, 2)
            o = xs[j // nsub, pl.ds((2 * (j % nsub) + ib) * R + 16 * g, 16), :].astype(f32) * dw
            d = o - jnp.sum(o, axis=-1, keepdims=True) * (1.0 / C)
            v = jnp.sum(d * d, axis=-1, keepdims=True) * (1.0 / (C * _A * _A)) + 1e-5 / (_A * _A)
            ln = d * jax.lax.rsqrt(v)
            blk = [ln[:, k * 128:(k + 1) * 128] for k in range(3)]
            if ib == 0:
                lns[g] = ln
                nodes = _forms(blk + blk, us)
            else:
                nodes = _forms([lns[g, :, pl.ds(k * 128, 128)] for k in range(3)] + blk, us)
            pin[NRES - 1, pl.ds(0, 8), :] = _zip(nodes[14 if ib else 8][0])
            for r, u in enumerate(un):
                if dep1[u] == (ib == 1):
                    fm[j % 3, r, pl.ds(8 * g, 8), :] = _zip(nodes[u][0])

        def step(j, q, c):
            def emit(o, z, sg):
                ib, jb = divmod(o, 3)
                col = jb * nb + c * 128
                th = jnp.tanh(z * (z * z + _K0))
                h = z * th + z if sg > 0 else z * th - z
                ssq[:, pl.ds(col, 128)] += (h * h).reshape(R // 8, 8, 128).sum(axis=0)
                unit(views[j // nsub] if j >= 0 else (None, prev), 2 * (j % nsub) + ib, col)[...] = _zip(h)

            r = prod_of[ORDER[q]]
            p = jnp.dot(_unpk(fm[j % 3, r]), _unpk(v1[r, c]), preferred_element_type=f32)
            absorb(ORDER, q, p, tot.at[c], emit)

        for t in range(15 * nj if last is None else 15 * (last + 2) + max(OFFS)):
            for c in range(4):
                jj, q = divmod(t - OFFS[c], 15)
                if jj - 1 >= first and (last is None or jj - 1 <= last):
                    step(jj - 1, q, c)
            for gg, tq in enumerate(LNT):
                if tq == t % 15 and t // 15 < nj:
                    norm_piece(t // 15, gg)

    for cp in w1_copies:
        cp.start()
    x_step(0).start()
    ssq[...] = jnp.zeros_like(ssq)
    fm[...] = jnp.zeros_like(fm)
    tot[...] = jnp.zeros_like(tot)
    for cp in w1_copies:
        cp.wait()
    for c in range(4):
        def w1_block(idx):
            q, col = divmod((idx % 3) * nb + c * 128, C)
            return pool[1, 0, pl.ds(q * C + (idx // 3) * 128, 128), pl.ds(col, 128)].astype(f32)
        for r in range(15):
            v1[r, c] = _pk(_weight_forms(w1_block, _SCHEME["v"][r]))

    def phase1(i, carry):
        tiles = [i * TPS + e for e in range(TPS)]
        views = [(ring(t), resident(1, t)) for t in tiles]
        prev, pin = resident(1, jnp.maximum(tiles[0] - 1, 0)), resident(2, tiles[-1])
        xs = pool.at[i & 1, pl.ds(2 - TPS, TPS)]
        for t in tiles:
            if_streamed(t - NSTG, lambda: h_out(t - NSTG).wait())
        x_step(i).wait()
        expand(xs, views, prev, pin, -2, None)
        for t in tiles:
            if_streamed(t, lambda: h_out(t).start(priority=HP))

        @pl.when(i + 2 < n1)
        def _():
            x_step(i + 2).start()

        @pl.when(i + 2 == n1)
        def _():
            w2_copy.start()
        return carry

    x_step(1).start()
    jax.lax.fori_loop(0, n1, phase1, 0)
    expand(None, [], resident(1, nt - 1), None, -2, -1)

    gx = jnp.sqrt(jnp.sum(ssq[...], axis=0, keepdims=True) * (_HS * _HS) + 1e-6)
    nx = gx / (jnp.mean(gx, axis=-1, keepdims=True) + 1e-6)
    scale = (g_ref[...].astype(f32).reshape(1, C4) * nx + 1.0) * _HS
    w2_copy.wait()
    for c in range(4):
        rows = [k * nb + c * 128 for k in range(3)]
        col = [jnp.broadcast_to(scale[:, r0:r0 + 128], (128, 128)).T for r0 in rows]

        def w2_block(idx):
            return w2_buf[pl.ds(rows[idx // 3], 128), pl.ds((idx % 3) * 128, 128)].astype(f32) * col[idx // 3]
        for r in range(15):
            v2[r, c] = _pk(_weight_forms(w2_block, _SCHEME["v"][r]))
    bias[...] = jnp.dot(jnp.broadcast_to(b_ref[...].astype(f32).reshape(1, C4), (8, C4)).astype(bf16), w2_buf[...], preferred_element_type=f32)

    def fetch(t):
        @pl.when(t + 2 < nt)
        def _():
            o_tile(t + 2).wait()

        @pl.when(t < nt - TPS)
        def _():
            x_tile(t).wait()

        if_streamed(t, lambda: h_in(t).wait())

    def phase2(i, carry):
        t = nt - 1 - i
        views = (ring(t), resident(3, t))
        xt, ot = pool.at[xside, t & 1], pool.at[1 - xside, t & 1]

        @pl.when(tab_ref[4, t] != -2)
        def _():
            fetch(t)

        def operand(j, r, c):
            acc = None
            for idx in np.argsort(-ucoef[r], kind="stable"):
                if ucoef[r][idx]:
                    ib, kb = divmod(int(idx), 3)
                    v = _unpk(unit(views, 2 * j + ib, kb * nb + c * 128)[...]).astype(f32)
                    acc = v if acc is None else (acc + v if ucoef[r][idx] > 0 else acc - v)
            return _unpk(_zip(acc))

        def step(j, q):
            def emit(o, y, sg):
                ib, jb = divmod(o, 3)
                rows, cols = pl.ds((2 * j + ib) * R, R), pl.ds(jb * 128, 128)
                base = _unzip(pltpu.bitcast(xt[rows, cols], jnp.uint32)) + bias[0:1, cols]
                ot[rows, cols] = _unpk(_zip(base + y if sg > 0 else base - y))

            r = prod_of[ORDER2[q]]
            p = [jnp.dot(operand(j, r, c), _unpk(v2[r, c]), preferred_element_type=f32) for c in range(4)]
            absorb(ORDER2, q, (p[0] + p[1]) + (p[2] + p[3]), tot.at[0], emit)

        for j in range(nsub):
            for q in range(15):
                step(j, q)
        o_tile(t).start()

        @pl.when(t >= 2)
        def _():
            x_tile(t - 2).start()

        if_streamed(t - NSTG, lambda: h_in(t - NSTG).start(priority=1))
        return carry

    def segment(m, carry):
        @pl.when(m > 0)
        def _():
            t = nt - 1 - tab_ref[6, m]
            fetch(t)
            expand(pool.at[xside, pl.ds(t & 1, 1)], [(ring(t), resident(3, t))], None, resident(5, t), 0, nsub - 1)

        return jax.lax.fori_loop(tab_ref[6, m], tab_ref[6, m + 1], phase2, carry)

    jax.lax.fori_loop(0, len(REDO) + 1, segment, 0)
    o_tile(1).wait()
    o_tile(0).wait()


@jax.jit
def pallas_standalone__modern_conv_block_slak__vision_kernel(x, dw, w1, w2, grn_g, grn_b):
    B, H, W, C = x.shape
    c4 = 4 * C
    assert B == 1 and dw.shape == (1, 1, C) and C == 384 and w1.shape == (C, c4) and TM == c4
    nt = H * W // TM
    nsub = TM // (2 * R)
    nstr = 2 * nsub * (c4 // 128) - NRES
    assert TPS == 2 and nt * TM == H * W and nt & 1 == 0 and nsub % 3 == 0 and NRES >= 4 * (c4 // 128)
    table, nkept, nsent = _placement(nt, nstr)
    hbm = pl.BlockSpec(memory_space=pl.ANY)
    vmem = pl.BlockSpec(memory_space=pltpu.VMEM)
    out, _ = pl.pallas_call(
        functools.partial(_body, nt=nt),
        in_specs=[hbm, vmem, hbm, hbm, vmem, vmem, pl.BlockSpec(memory_space=pltpu.SMEM)],
        out_specs=[hbm, hbm],
        out_shape=[
            jax.ShapeDtypeStruct((nt, TM, C), x.dtype),
            jax.ShapeDtypeStruct((nsent, nstr, R // 2, 128), jnp.uint32),
        ],
        scratch_shapes=[
            pltpu.VMEM((2, 2, TM, C), x.dtype),
            pltpu.VMEM((nkept * NRES + NSTG * nstr, R // 2, 128), jnp.uint32),
            pltpu.VMEM((15, 4, 64, 128), jnp.uint32),
            pltpu.VMEM((15, 4, 64, 128), jnp.uint32),
            pltpu.VMEM((8, c4), jnp.float32),
            pltpu.VMEM((3, 15, R // 2, 128), jnp.uint32),
            pltpu.VMEM((4, 10, R, 128), jnp.float32),
            pltpu.VMEM((R // 16, 16, C), jnp.float32),
            pltpu.VMEM((8, C), jnp.float32),
            pltpu.SemaphoreType.DMA((NSTG,)),
            pltpu.SemaphoreType.DMA((2,)),
            pltpu.SemaphoreType.DMA((2,)),
            pltpu.SemaphoreType.DMA((4,)),
        ],
        compiler_params=pltpu.CompilerParams(vmem_limit_bytes=128 * 1024 * 1024, flags=FLAGS, disable_bounds_checks=NOBC),
    )(x.reshape(nt, TM, C), dw.reshape(1, C), w1, w2, grn_g, grn_b, table)
    return out.reshape(B, H, W, C)
```

```python
import functools

import jax
import jax.numpy as jnp
import numpy as np
from jax.experimental import pallas as pl
from jax.experimental.pallas import tpu as pltpu

TM = 1536
R = 64
NRES = 65
NSTG = 6
REDO = (70, 45, 20)
OCUT = 10

ORDER1 = (14, 13, 7, 15, 11, 8, 12, 10, 4, 1, 5, 9, 6, 2, 3)
OFFS = (0, 1, 7, 8)
LNT = (2, 3, 4, 5, 7, 8, 9, 12)
ORDER2 = (7, 15, 14, 12, 13, 4, 10, 11, 5, 9, 1, 8, 6, 3, 2)

_C0 = float(np.sqrt(2.0 / np.pi))
_A = (0.044715 * _C0) ** (1.0 / 3.0)
_K0 = _C0 / _A
_HS = 0.5 / _A

US = [(0, 1, 3, -1), (6, 1, 5, -1), (1, 1, 2, -1), (1, 1, 4, -1), (8, 1, 4, -1), (0, 1, 1, 1), (7, 1, 2, 1),
      (0, 1, 4, 1), (6, -1, 13, 1), (0, 1, 7, -1), (8, 1, 15, 1)]
UN = [5, 16, 15, 2, 13, 9, 4, 6, 11, 10, 0, 8, 12, 14, 7]
WS = [(0, 1, 2, -1), (0, 1, 1, 1), (0, 1, 3, 1), (6, 1, 3, 1), (9, 1, 5, -1), (1, 1, 8, 1), (10, 1, 4, 1),
      (11, 1, 4, 1), (13, 1, 5, -1), (1, 1, 12, 1)]
WN = [5, 12, 10, 2, 11, 7, 13, 3, 1, 14, 8, 15, 6, 4, 9]
V = [[0, 0, -1, 0, 0, 0, 0, 0, 1], [0, 0, 0, 0, 0, 0, 0, 1, 0], [0, 0, -1, 0, 0, 0, 0, -1, 0],
     [0, 0, 0, 0, 0, 1, 1, 0, 1], [0, 1, 0, 1, -1, 0, 0, -1, 0], [0, 0, 0, 1, 0, 0, 0, 0, 0],
     [0, -1, 0, 0, 1, 1, 0, 1, 0], [-1, 0, 0, 0, 0, 0, 1, 0, 0], [0, 0, 0, -1, 1, 0, 0, 1, 0],
     [0, 0, 0, 0, 0, 1, 0, 0, 0], [1, -1, 1, -1, 1, 0, 0, 1, 0], [0, 0, 0, 0, 0, -1, 0, -1, 0],
     [0, 0, 0, 0, 0, 0, 1, 0, 0], [0, 1, 0, 0, 0, 0, 0, -1, 0], [0, 0, -1, 0, 0, 0, -1, 0, 0]]


def _addsub(a, sa, b, sb):
    if sa == sb:
        return a + b, sa
    return (a - b, 1) if sa > 0 else (b - a, 1)


def _left_nodes(blocks):
    nodes = [(blk, 1) for blk in blocks]
    for a, sa, b, sb in US:
        nodes.append(_addsub(nodes[a][0], sa * nodes[a][1], nodes[b][0], sb * nodes[b][1]))
    return nodes


def _right_operand(block, coefs):
    acc = None
    for idx, c in enumerate(coefs):
        if c:
            t = block(idx)
            acc = (t if c > 0 else -t) if acc is None else (acc + t if c > 0 else acc - t)
    return acc


_UNODES = _left_nodes(list(np.eye(6, dtype=int)))
_UCOEF = [_UNODES[u][0] for u in UN]
_USGN = [_UNODES[u][1] for u in UN]
_PRODUCT = {n: r for r, n in enumerate(WN)}
_FEEDS = {n: [(6 + t, s) for t, (a, sa, b, sb) in enumerate(WS) for m, s in ((a, sa), (b, sb)) if m == n]
          for n in range(6 + len(WS))}


def _absorb(order, q, p, sums, emit):
    sign = {}
    for n in order:
        sign[n] = _USGN[_PRODUCT[n]]
        for src, s in _FEEDS[n]:
            sign[n] = _addsub(0, sign[n], 0, s * sign[src])[1]
    n, done = order[q], order[:q + 1]
    acc = (p, _USGN[_PRODUCT[n]])
    for src, s in _FEEDS[n]:
        acc = _addsub(*acc, sums[src - 6], s * sign[src])
    if n < 6:
        emit(n, *acc)
        return
    keep = any(src == n for m in order[q + 1:] for src, _ in _FEEDS[m])
    for o in range(6):
        mine = [s for src, s in _FEEDS[o] if src == n]
        if o in _PRODUCT or not mine:
            continue
        if all(src in done for src, _ in _FEEDS[o]):
            res = (acc[0], acc[1] * mine[0])
            for src, s in _FEEDS[o]:
                if src != n:
                    res = _addsub(*res, sums[src - 6], s * sign[src])
            emit(o, *res)
        else:
            keep = True
    if keep:
        sums[n - 6] = acc[0]


def _to_words(v):
    return pltpu.bitcast(v.astype(jnp.bfloat16), jnp.uint32)


def _from_words(w):
    return pltpu.bitcast(w, jnp.bfloat16)


def _zip(v):
    half = [jnp.concatenate([v[16 * i + 8 * e:16 * i + 8 * e + 8] for i in range(v.shape[0] // 16)], axis=0)
            for e in range(2)]
    return pltpu.pack_elementwise(half, packed_dtype=jnp.bfloat16)


def _unzip(w):
    half = [pltpu.unpack_elementwise(w, index=e, packed_dtype=jnp.bfloat16, unpacked_dtype=jnp.float32)
            for e in range(2)]
    return jnp.concatenate([half[e][8 * i:8 * i + 8] for i in range(w.shape[0] // 8) for e in range(2)], axis=0)


_RING, _HOME1, _ALIAS1, _HOME2, _HBM, _ALIAS2, _CUTS, _SLOT = range(8)


def _placement(nt, nstr):
    assert all(t + 4 < nt - NSTG and t + 1 not in REDO and t + 4 not in REDO for t in REDO)
    kept = [t for t in range(nt) if t not in REDO]
    sent = [t for t in kept if t < nt - NSTG]
    base = {t: k * NRES for k, t in enumerate(kept)}
    home1 = [base[t + 4] if t in REDO else base[t] for t in range(nt)]
    home2 = [base[t + 1] if t in REDO else base[t] for t in range(nt)]
    ring = [len(kept) * NRES + (t % NSTG) * nstr for t in range(nt)]
    hbm = [sent.index(t) if t in sent else (-2 if t in REDO else -1) for t in range(nt)]
    cuts = [0] + sorted(nt - 1 - t for t in REDO)
    cuts += [nt] * (nt - len(cuts))
    slot = [t % NSTG for t in range(nt)]
    return np.array([ring, home1, home1, home2, hbm, home2, cuts, slot], np.int32), len(kept), len(sent)


def _body(x_hbm, dw_ref, w1_hbm, w2_hbm, g_ref, b_ref, tab_ref, o_hbm, h_hbm,
          pool, hbuf, v1, v2, ssq, fm, tot, lns, bias, hsem, xsem, osem, wsem, *, nt):
    f32, bf16 = jnp.float32, jnp.bfloat16
    C, C4 = w1_hbm.shape
    nb = C4 // 3
    ncol = C4 // 128
    nsub = TM // (2 * R)
    nstr = 2 * nsub * ncol - NRES
    n1 = nt // 2
    xside = (n1 - 1) % 2

    def ring(t):
        return hbuf.at[pl.ds(tab_ref[_RING, t], nstr)]

    def resident(row, t):
        return hbuf.at[pl.ds(tab_ref[row, t], NRES)]

    def unit(views, blk, col):
        u = blk * ncol + col // 128
        return views[0].at[u] if u < nstr else views[1].at[u - nstr]

    def if_streamed(t, fn):
        @pl.when(jnp.logical_and(t >= 0, tab_ref[_HBM, jnp.maximum(t, 0)] >= 0))
        def _():
            fn()

    def h_out(t):
        return pltpu.make_async_copy(ring(t), h_hbm.at[tab_ref[_HBM, t]], hsem.at[tab_ref[_SLOT, t]])

    def h_in(t):
        return pltpu.make_async_copy(h_hbm.at[tab_ref[_HBM, t]], ring(t), hsem.at[tab_ref[_SLOT, t]])

    def x_step(i):
        return pltpu.make_async_copy(x_hbm.at[pl.ds(2 * i, 2)], pool.at[i & 1], xsem.at[i & 1])

    def x_tile(t):
        return pltpu.make_async_copy(x_hbm.at[t], pool.at[xside, t & 1], xsem.at[t & 1])

    def o_part(t, e):
        rows = pl.ds(OCUT * 2 * R, TM - OCUT * 2 * R) if e else pl.ds(0, OCUT * 2 * R)
        return pltpu.make_async_copy(pool.at[1 - xside, t & 1, rows], o_hbm.at[t, rows], osem.at[(t & 1) * 2 + e])

    w1_copies = [pltpu.make_async_copy(w1_hbm.at[:, pl.ds(q * C, C)], pool.at[1, 0, pl.ds(q * C, C)], wsem.at[q])
                 for q in range(4)]
    w2_buf = pool.at[1 - xside, 0]
    w2_copy = pltpu.make_async_copy(w2_hbm, w2_buf, wsem.at[0])

    def expand(xs, views, prev, pin, first, last):
        dw = dw_ref[...].astype(f32)
        nj = len(views) * nsub

        def norm_piece(j, gg):
            g, ib = divmod(gg, 2)
            o = xs[j // nsub, pl.ds((2 * (j % nsub) + ib) * R + 16 * g, 16), :].astype(f32) * dw
            d = o - jnp.sum(o, axis=-1, keepdims=True) * (1.0 / C)
            v = jnp.sum(d * d, axis=-1, keepdims=True) * (1.0 / (C * _A * _A)) + 1e-5 / (_A * _A)
            ln = d * jax.lax.rsqrt(v)
            blk = [ln[:, k * 128:(k + 1) * 128] for k in range(3)]
            if ib == 0:
                lns[g] = ln
                nodes = _left_nodes(blk + blk)
            else:
                nodes = _left_nodes([lns[g, :, pl.ds(k * 128, 128)] for k in range(3)] + blk)
            pin[NRES - 1, pl.ds(0, 8), :] = _zip(nodes[14 if ib else 8][0])
            for r, u in enumerate(UN):
                if bool(_UCOEF[r][3:].any()) == (ib == 1):
                    fm[j % 3, r, pl.ds(8 * g, 8), :] = _zip(nodes[u][0])

        def step(j, q, c):
            def emit(o, z, sg):
                ib, jb = divmod(o, 3)
                col = jb * nb + c * 128
                th = jnp.tanh(z * (z * z + _K0))
                h = z * th + z if sg > 0 else z * th - z
                ssq[:, pl.ds(col, 128)] += (h * h).reshape(R // 8, 8, 128).sum(axis=0)
                unit(views[j // nsub] if j >= 0 else (None, prev), 2 * (j % nsub) + ib, col)[...] = _zip(h)

            r = _PRODUCT[ORDER1[q]]
            p = jnp.dot(_from_words(fm[j % 3, r]), _from_words(v1[r, c]), preferred_element_type=f32)
            _absorb(ORDER1, q, p, tot.at[c], emit)

        for t in range(15 * nj if last is None else 15 * (last + 2) + max(OFFS)):
            for c in range(4):
                jj, q = divmod(t - OFFS[c], 15)
                if jj - 1 >= first and (last is None or jj - 1 <= last):
                    step(jj - 1, q, c)
            for gg, tq in enumerate(LNT):
                if tq == t % 15 and t // 15 < nj:
                    norm_piece(t // 15, gg)

    for cp in w1_copies:
        cp.start()
    x_step(0).start()
    ssq[...] = jnp.zeros_like(ssq)
    fm[...] = jnp.zeros_like(fm)
    tot[...] = jnp.zeros_like(tot)
    for cp in w1_copies:
        cp.wait()
    for c in range(4):
        def w1_block(idx):
            q, col = divmod((idx % 3) * nb + c * 128, C)
            return pool[1, 0, pl.ds(q * C + (idx // 3) * 128, 128), pl.ds(col, 128)].astype(f32)
        for r in range(15):
            v1[r, c] = _to_words(_right_operand(w1_block, V[r]))

    def phase1(i, carry):
        tiles = [2 * i, 2 * i + 1]
        views = [(ring(t), resident(_HOME1, t)) for t in tiles]
        prev, pin = resident(_HOME1, jnp.maximum(tiles[0] - 1, 0)), resident(_ALIAS1, tiles[-1])
        xs = pool.at[i & 1]
        for t in tiles:
            if_streamed(t - NSTG, lambda: h_out(t - NSTG).wait())
        x_step(i).wait()
        expand(xs, views, prev, pin, -2, None)
        for t in tiles:
            if_streamed(t, lambda: h_out(t).start())

        @pl.when(i + 2 < n1)
        def _():
            x_step(i + 2).start()

        @pl.when(i + 2 == n1)
        def _():
            w2_copy.start()
        return carry

    x_step(1).start()
    jax.lax.fori_loop(0, n1, phase1, 0)
    expand(None, [], resident(_HOME1, nt - 1), None, -2, -1)

    gx = jnp.sqrt(jnp.sum(ssq[...], axis=0, keepdims=True) * (_HS * _HS) + 1e-6)
    nx = gx / (jnp.mean(gx, axis=-1, keepdims=True) + 1e-6)
    scale = (g_ref[...].astype(f32).reshape(1, C4) * nx + 1.0) * _HS
    w2_copy.wait()
    for c in range(4):
        rows = [k * nb + c * 128 for k in range(3)]
        col = [jnp.broadcast_to(scale[:, r0:r0 + 128], (128, 128)).T for r0 in rows]

        def w2_block(idx):
            return w2_buf[pl.ds(rows[idx // 3], 128), pl.ds((idx % 3) * 128, 128)].astype(f32) * col[idx // 3]
        for r in range(15):
            v2[r, c] = _to_words(_right_operand(w2_block, V[r]))
    shift = jnp.broadcast_to(b_ref[...].astype(f32).reshape(1, C4), (8, C4)).astype(bf16)
    bias[...] = jnp.dot(shift, w2_buf[...], preferred_element_type=f32)

    def fetch(t):
        @pl.when(t + 2 < nt)
        def _():
            o_part(t + 2, 0).wait()
            o_part(t + 2, 1).wait()

        @pl.when(t < nt - 2)
        def _():
            x_tile(t).wait()

        if_streamed(t, lambda: h_in(t).wait())

    def phase2(i, carry):
        t = nt - 1 - i
        views = (ring(t), resident(_HOME2, t))
        xt, ot = pool.at[xside, t & 1], pool.at[1 - xside, t & 1]

        @pl.when(tab_ref[_HBM, t] != -2)
        def _():
            fetch(t)

        def operand(j, r, c):
            acc = None
            for idx in np.argsort(-_UCOEF[r], kind="stable"):
                if _UCOEF[r][idx]:
                    ib, kb = divmod(int(idx), 3)
                    v = _from_words(unit(views, 2 * j + ib, kb * nb + c * 128)[...]).astype(f32)
                    acc = v if acc is None else (acc + v if _UCOEF[r][idx] > 0 else acc - v)
            return _from_words(_zip(acc))

        def step(j, q):
            def emit(o, y, sg):
                ib, jb = divmod(o, 3)
                rows, cols = pl.ds((2 * j + ib) * R, R), pl.ds(jb * 128, 128)
                base = _unzip(pltpu.bitcast(xt[rows, cols], jnp.uint32)) + bias[0:1, cols]
                ot[rows, cols] = _from_words(_zip(base + y if sg > 0 else base - y))

            r = _PRODUCT[ORDER2[q]]
            p = [jnp.dot(operand(j, r, c), _from_words(v2[r, c]), preferred_element_type=f32) for c in range(4)]
            _absorb(ORDER2, q, (p[0] + p[1]) + (p[2] + p[3]), tot.at[0], emit)

        for j in range(nsub):
            for q in range(15):
                step(j, q)
            if j + 1 == OCUT:
                o_part(t, 0).start()
        o_part(t, 1).start()

        @pl.when(t >= 2)
        def _():
            x_tile(t - 2).start()

        if_streamed(t - NSTG, lambda: h_in(t - NSTG).start(priority=1))
        return carry

    def segment(m, carry):
        @pl.when(m > 0)
        def _():
            t = nt - 1 - tab_ref[_CUTS, m]
            fetch(t)
            expand(pool.at[xside, pl.ds(t & 1, 1)], [(ring(t), resident(_HOME2, t))], None, resident(_ALIAS2, t),
                   0, nsub - 1)

        return jax.lax.fori_loop(tab_ref[_CUTS, m], tab_ref[_CUTS, m + 1], phase2, carry)

    jax.lax.fori_loop(0, len(REDO) + 1, segment, 0)
    for t in (1, 0):
        for e in (0, 1):
            o_part(t, e).wait()


@jax.jit
def pallas_standalone__modern_conv_block_slak__vision_kernel(x, dw, w1, w2, grn_g, grn_b):
    B, H, W, C = x.shape
    c4 = 4 * C
    assert B == 1 and dw.shape == (1, 1, C) and C == 384 and w1.shape == (C, c4) and TM == c4
    nt = H * W // TM
    nsub = TM // (2 * R)
    nstr = 2 * nsub * (c4 // 128) - NRES
    assert nt * TM == H * W and nt % 2 == 0 and nsub % 3 == 0 and NRES >= 4 * (c4 // 128)
    table, nkept, nsent = _placement(nt, nstr)
    hbm = pl.BlockSpec(memory_space=pl.ANY)
    vmem = pl.BlockSpec(memory_space=pltpu.VMEM)
    out, _ = pl.pallas_call(
        functools.partial(_body, nt=nt),
        in_specs=[hbm, vmem, hbm, hbm, vmem, vmem, pl.BlockSpec(memory_space=pltpu.SMEM)],
        out_specs=[hbm, hbm],
        out_shape=[
            jax.ShapeDtypeStruct((nt, TM, C), x.dtype),
            jax.ShapeDtypeStruct((nsent, nstr, R // 2, 128), jnp.uint32),
        ],
        scratch_shapes=[
            pltpu.VMEM((2, 2, TM, C), x.dtype),
            pltpu.VMEM((nkept * NRES + NSTG * nstr, R // 2, 128), jnp.uint32),
            pltpu.VMEM((15, 4, 64, 128), jnp.uint32),
            pltpu.VMEM((15, 4, 64, 128), jnp.uint32),
            pltpu.VMEM((8, c4), jnp.float32),
            pltpu.VMEM((3, 15, R // 2, 128), jnp.uint32),
            pltpu.VMEM((4, 10, R, 128), jnp.float32),
            pltpu.VMEM((R // 16, 16, C), jnp.float32),
            pltpu.VMEM((8, C), jnp.float32),
            pltpu.SemaphoreType.DMA((NSTG,)),
            pltpu.SemaphoreType.DMA((2,)),
            pltpu.SemaphoreType.DMA((4,)),
            pltpu.SemaphoreType.DMA((4,)),
        ],
        compiler_params=pltpu.CompilerParams(vmem_limit_bytes=128 * 1024 * 1024, disable_bounds_checks=True),
    )(x.reshape(nt, TM, C), dw.reshape(1, C), w1, w2, grn_g, grn_b, table)
    return out.reshape(B, H, W, C)
```

```python
import functools

import jax
import jax.numpy as jnp
import numpy as np
from jax.experimental import pallas as pl
from jax.experimental.pallas import tpu as pltpu

TM = 1536
R = 64
NRES = 65
NSTG = 6
REDO = (70, 45, 20)
OCUT = 10

ORDER1 = (14, 13, 15, 7, 11, 12, 8, 10, 1, 9, 4, 3, 6, 2, 5)
OFFS = (0, 1, 7, 8)
LNT = (0, 1, 2, 6, 7, 8, 11, 12)
ORDER2 = (7, 15, 14, 12, 13, 4, 10, 11, 5, 9, 1, 8, 6, 3, 2)

_C0 = float(np.sqrt(2.0 / np.pi))
_A = (0.044715 * _C0) ** (1.0 / 3.0)
_K0 = _C0 / _A
_HS = 0.5 / _A

US = [(0, 1, 3, -1), (6, 1, 5, -1), (1, 1, 2, -1), (1, 1, 4, -1), (8, 1, 4, -1), (0, 1, 1, 1), (7, 1, 2, 1),
      (0, 1, 4, 1), (6, -1, 13, 1), (0, 1, 7, -1), (8, 1, 15, 1)]
UN = [5, 16, 15, 2, 13, 9, 4, 6, 11, 10, 0, 8, 12, 14, 7]
WS = [(0, 1, 2, -1), (0, 1, 1, 1), (0, 1, 3, 1), (6, 1, 3, 1), (9, 1, 5, -1), (1, 1, 8, 1), (10, 1, 4, 1),
      (11, 1, 4, 1), (13, 1, 5, -1), (1, 1, 12, 1)]
WN = [5, 12, 10, 2, 11, 7, 13, 3, 1, 14, 8, 15, 6, 4, 9]
V = [[0, 0, -1, 0, 0, 0, 0, 0, 1], [0, 0, 0, 0, 0, 0, 0, 1, 0], [0, 0, -1, 0, 0, 0, 0, -1, 0],
     [0, 0, 0, 0, 0, 1, 1, 0, 1], [0, 1, 0, 1, -1, 0, 0, -1, 0], [0, 0, 0, 1, 0, 0, 0, 0, 0],
     [0, -1, 0, 0, 1, 1, 0, 1, 0], [-1, 0, 0, 0, 0, 0, 1, 0, 0], [0, 0, 0, -1, 1, 0, 0, 1, 0],
     [0, 0, 0, 0, 0, 1, 0, 0, 0], [1, -1, 1, -1, 1, 0, 0, 1, 0], [0, 0, 0, 0, 0, -1, 0, -1, 0],
     [0, 0, 0, 0, 0, 0, 1, 0, 0], [0, 1, 0, 0, 0, 0, 0, -1, 0], [0, 0, -1, 0, 0, 0, -1, 0, 0]]


def _addsub(a, sa, b, sb):
    if sa == sb:
        return a + b, sa
    return (a - b, 1) if sa > 0 else (b - a, 1)


def _left_nodes(blocks):
    nodes = [(blk, 1) for blk in blocks]
    for a, sa, b, sb in US:
        nodes.append(_addsub(nodes[a][0], sa * nodes[a][1], nodes[b][0], sb * nodes[b][1]))
    return nodes


def _right_operand(block, coefs):
    acc = None
    for idx, c in enumerate(coefs):
        if c:
            t = block(idx)
            acc = (t if c > 0 else -t) if acc is None else (acc + t if c > 0 else acc - t)
    return acc


_UNODES = _left_nodes(list(np.eye(6, dtype=int)))
_UCOEF = [_UNODES[u][0] for u in UN]
_USGN = [_UNODES[u][1] for u in UN]
_EARLY = [r for r in range(15) if not _UCOEF[r][3:].any()]
_LATE = [r for r in range(15) if r not in _EARLY]
_PAIRS = [rs[i:i + 2] for rs in (_EARLY, _LATE) for i in range(0, len(rs), 2)]
_PRODUCT = {n: r for r, n in enumerate(WN)}
_FEEDS = {n: [(6 + t, s) for t, (a, sa, b, sb) in enumerate(WS) for m, s in ((a, sa), (b, sb)) if m == n]
          for n in range(6 + len(WS))}


def _absorb(order, q, p, sums, emit):
    sign = {}
    for n in order:
        sign[n] = _USGN[_PRODUCT[n]]
        for src, s in _FEEDS[n]:
            sign[n] = _addsub(0, sign[n], 0, s * sign[src])[1]
    n, done = order[q], order[:q + 1]
    acc = (p, _USGN[_PRODUCT[n]])
    for src, s in _FEEDS[n]:
        acc = _addsub(*acc, sums[src - 6], s * sign[src])
    if n < 6:
        emit(n, *acc)
        return
    keep = any(src == n for m in order[q + 1:] for src, _ in _FEEDS[m])
    for o in range(6):
        mine = [s for src, s in _FEEDS[o] if src == n]
        if o in _PRODUCT or not mine:
            continue
        if all(src in done for src, _ in _FEEDS[o]):
            res = (acc[0], acc[1] * mine[0])
            for src, s in _FEEDS[o]:
                if src != n:
                    res = _addsub(*res, sums[src - 6], s * sign[src])
            emit(o, *res)
        else:
            keep = True
    if keep:
        sums[n - 6] = acc[0]


def _to_words(v):
    return pltpu.bitcast(v.astype(jnp.bfloat16), jnp.uint32)


def _from_words(w):
    return pltpu.bitcast(w, jnp.bfloat16)


def _fold(v):
    return jnp.concatenate([jnp.concatenate([v[i:i + 8], v[i + 8:i + 16]], axis=1)
                            for i in range(0, v.shape[0], 16)], axis=0)


def _unfold(v):
    return jnp.concatenate([v[i:i + 8, e:e + 128] for i in range(0, v.shape[0], 8) for e in (0, 128)], axis=0)


_RING, _HOME1, _ALIAS1, _HOME2, _HBM, _ALIAS2, _CUTS, _SLOT = range(8)


def _placement(nt, nstr):
    assert all(t + 4 < nt - NSTG and t + 1 not in REDO and t + 4 not in REDO for t in REDO)
    kept = [t for t in range(nt) if t not in REDO]
    sent = [t for t in kept if t < nt - NSTG]
    base = {t: k * NRES for k, t in enumerate(kept)}
    home1 = [base[t + 4] if t in REDO else base[t] for t in range(nt)]
    home2 = [base[t + 1] if t in REDO else base[t] for t in range(nt)]
    ring = [len(kept) * NRES + (t % NSTG) * nstr for t in range(nt)]
    hbm = [sent.index(t) if t in sent else (-2 if t in REDO else -1) for t in range(nt)]
    cuts = [0] + sorted(nt - 1 - t for t in REDO)
    cuts += [nt] * (nt - len(cuts))
    slot = [t % NSTG for t in range(nt)]
    return np.array([ring, home1, home1, home2, hbm, home2, cuts, slot], np.int32), len(kept), len(sent)


def _body(x_hbm, dw_ref, w1_hbm, w2_hbm, g_ref, b_ref, tab_ref, o_hbm, h_hbm,
          pool, hbuf, v1, v2, ssq, fm, tot, lns, bias, hsem, xsem, osem, wsem, *, nt):
    f32, bf16 = jnp.float32, jnp.bfloat16
    C, C4 = w1_hbm.shape
    nb = C4 // 3
    ncol = C4 // 128
    nsub = TM // (2 * R)
    nstr = 2 * nsub * ncol - NRES
    n1 = nt // 2
    xside = (n1 - 1) % 2

    def ring(t):
        return hbuf.at[pl.ds(tab_ref[_RING, t], nstr)]

    def resident(row, t):
        return hbuf.at[pl.ds(tab_ref[row, t], NRES)]

    def unit(views, blk, col):
        u = blk * ncol + col // 128
        return views[0].at[u] if u < nstr else views[1].at[u - nstr]

    def if_streamed(t, fn):
        @pl.when(jnp.logical_and(t >= 0, tab_ref[_HBM, jnp.maximum(t, 0)] >= 0))
        def _():
            fn()

    def h_out(t):
        return pltpu.make_async_copy(ring(t), h_hbm.at[tab_ref[_HBM, t]], hsem.at[tab_ref[_SLOT, t]])

    def h_in(t):
        return pltpu.make_async_copy(h_hbm.at[tab_ref[_HBM, t]], ring(t), hsem.at[tab_ref[_SLOT, t]])

    def x_step(i):
        return pltpu.make_async_copy(x_hbm.at[pl.ds(2 * i, 2)], pool.at[i & 1], xsem.at[i & 1])

    def x_tile(t):
        return pltpu.make_async_copy(x_hbm.at[t], pool.at[xside, t & 1], xsem.at[t & 1])

    def o_part(t, e):
        rows = pl.ds(OCUT * 2 * R, TM - OCUT * 2 * R) if e else pl.ds(0, OCUT * 2 * R)
        return pltpu.make_async_copy(pool.at[1 - xside, t & 1, rows], o_hbm.at[t, rows], osem.at[(t & 1) * 2 + e])

    w1_copies = [pltpu.make_async_copy(w1_hbm.at[:, pl.ds(q * C, C)], pool.at[1, 0, pl.ds(q * C, C)], wsem.at[q])
                 for q in range(4)]
    w2_buf = pool.at[1 - xside, 0]
    w2_copy = pltpu.make_async_copy(w2_hbm, w2_buf, wsem.at[0])

    def expand(xs, views, prev, pin, first, last):
        dw = dw_ref[...].astype(f32)
        nj = len(views) * nsub

        def norm_piece(j, gg):
            g, ib = divmod(gg, 2)
            o = xs[j // nsub, pl.ds((2 * (j % nsub) + ib) * R + 16 * g, 16), :].astype(f32) * dw
            d = o - jnp.sum(o, axis=-1, keepdims=True) * (1.0 / C)
            v = jnp.sum(d * d, axis=-1, keepdims=True) * (1.0 / (C * _A * _A)) + 1e-5 / (_A * _A)
            ln = d * jax.lax.rsqrt(v)
            blk = [ln[:, k * 128:(k + 1) * 128] for k in range(3)]
            if ib == 0:
                lns[g] = ln
                nodes = _left_nodes(blk + blk)
            else:
                nodes = _left_nodes([lns[g, :, pl.ds(k * 128, 128)] for k in range(3)] + blk)
            pin[NRES - 1, pl.ds(0, 8), :] = _fold(nodes[14 if ib else 8][0]).astype(bf16)
            for k, pair in enumerate(_PAIRS):
                if bool(_UCOEF[pair[0]][3:].any()) == (ib == 1):
                    both = jnp.concatenate([nodes[UN[r]][0] for r in pair], axis=1)
                    fm[j % 3, k, pl.ds(8 * g, 8), pl.ds(0, both.shape[1])] = _to_words(both)

        def step(j, q, c):
            def emit(o, z, sg):
                ib, jb = divmod(o, 3)
                col = jb * nb + c * 128
                th = jnp.tanh(z * (z * z + _K0))
                h = z * th + z if sg > 0 else z * th - z
                ssq[:, pl.ds(col, 128)] += (h * h).reshape(R // 8, 8, 128).sum(axis=0)
                unit(views[j // nsub] if j >= 0 else (None, prev), 2 * (j % nsub) + ib, col)[...] = _fold(h).astype(bf16)

            r = _PRODUCT[ORDER1[q]]
            k, e = next((k, pair.index(r)) for k, pair in enumerate(_PAIRS) if r in pair)
            lhs = _from_words(fm[j % 3, k, :, pl.ds(128 * e, 128)])
            p = jnp.dot(lhs, _from_words(v1[r, c]), preferred_element_type=f32)
            _absorb(ORDER1, q, p, tot.at[c], emit)

        for t in range(15 * nj if last is None else 15 * (last + 2) + max(OFFS)):
            for c in range(4):
                jj, q = divmod(t - OFFS[c], 15)
                if jj - 1 >= first and (last is None or jj - 1 <= last):
                    step(jj - 1, q, c)
            for gg, tq in enumerate(LNT):
                if tq == t % 15 and t // 15 < nj:
                    norm_piece(t // 15, gg)

    for cp in w1_copies:
        cp.start()
    x_step(0).start()
    ssq[...] = jnp.zeros_like(ssq)
    fm[...] = jnp.zeros_like(fm)
    tot[...] = jnp.zeros_like(tot)
    for cp in w1_copies:
        cp.wait()
    for c in range(4):
        def w1_block(idx):
            q, col = divmod((idx % 3) * nb + c * 128, C)
            return pool[1, 0, pl.ds(q * C + (idx // 3) * 128, 128), pl.ds(col, 128)].astype(f32)
        for r in range(15):
            v1[r, c] = _to_words(_right_operand(w1_block, V[r]))

    def phase1(i, carry):
        tiles = [2 * i, 2 * i + 1]
        views = [(ring(t), resident(_HOME1, t)) for t in tiles]
        prev, pin = resident(_HOME1, jnp.maximum(tiles[0] - 1, 0)), resident(_ALIAS1, tiles[-1])
        xs = pool.at[i & 1]
        for t in tiles:
            if_streamed(t - NSTG, lambda: h_out(t - NSTG).wait())
        x_step(i).wait()
        expand(xs, views, prev, pin, -2, None)
        for t in tiles:
            if_streamed(t, lambda: h_out(t).start())

        @pl.when(i + 2 < n1)
        def _():
            x_step(i + 2).start()

        @pl.when(i + 2 == n1)
        def _():
            w2_copy.start()
        return carry

    x_step(1).start()
    jax.lax.fori_loop(0, n1, phase1, 0)
    expand(None, [], resident(_HOME1, nt - 1), None, -2, -1)

    gx = jnp.sqrt(jnp.sum(ssq[...], axis=0, keepdims=True) * (_HS * _HS) + 1e-6)
    nx = gx / (jnp.mean(gx, axis=-1, keepdims=True) + 1e-6)
    scale = (g_ref[...].astype(f32).reshape(1, C4) * nx + 1.0) * _HS
    w2_copy.wait()
    for c in range(4):
        rows = [k * nb + c * 128 for k in range(3)]
        col = [jnp.broadcast_to(scale[:, r0:r0 + 128], (128, 128)).T for r0 in rows]

        def w2_block(idx):
            return w2_buf[pl.ds(rows[idx // 3], 128), pl.ds((idx % 3) * 128, 128)].astype(f32) * col[idx // 3]
        for r in range(15):
            v2[r, c] = _to_words(_right_operand(w2_block, V[r]))
    shift = jnp.broadcast_to(b_ref[...].astype(f32).reshape(1, C4), (8, C4)).astype(bf16)
    bias[...] = jnp.dot(shift, w2_buf[...], preferred_element_type=f32)

    def fetch(t):
        @pl.when(t + 2 < nt)
        def _():
            o_part(t + 2, 0).wait()
            o_part(t + 2, 1).wait()

        @pl.when(t < nt - 2)
        def _():
            x_tile(t).wait()

        if_streamed(t, lambda: h_in(t).wait())

    def phase2(i, carry):
        t = nt - 1 - i
        views = (ring(t), resident(_HOME2, t))
        xt, ot = pool.at[xside, t & 1], pool.at[1 - xside, t & 1]

        @pl.when(tab_ref[_HBM, t] != -2)
        def _():
            fetch(t)

        def operand(j, r, c):
            acc = None
            for idx in np.argsort(-_UCOEF[r], kind="stable"):
                if _UCOEF[r][idx]:
                    ib, kb = divmod(int(idx), 3)
                    v = unit(views, 2 * j + ib, kb * nb + c * 128)[...].astype(f32)
                    acc = v if acc is None else (acc + v if _UCOEF[r][idx] > 0 else acc - v)
            return _unfold(acc).astype(bf16)

        def step(j, q):
            def emit(o, y, sg):
                ib, jb = divmod(o, 3)
                rows, cols = pl.ds((2 * j + ib) * R, R), pl.ds(jb * 128, 128)
                base = xt[rows, cols].astype(f32) + bias[0:1, cols]
                ot[rows, cols] = (base + y if sg > 0 else base - y).astype(bf16)

            r = _PRODUCT[ORDER2[q]]
            p = [jnp.dot(operand(j, r, c), _from_words(v2[r, c]), preferred_element_type=f32) for c in range(4)]
            _absorb(ORDER2, q, (p[0] + p[1]) + (p[2] + p[3]), tot.at[0], emit)

        for j in range(nsub):
            for q in range(15):
                step(j, q)
            if j + 1 == OCUT:
                o_part(t, 0).start()
        o_part(t, 1).start()

        @pl.when(t >= 2)
        def _():
            x_tile(t - 2).start()

        if_streamed(t - NSTG, lambda: h_in(t - NSTG).start(priority=1))
        return carry

    def segment(m, carry):
        @pl.when(m > 0)
        def _():
            t = nt - 1 - tab_ref[_CUTS, m]
            fetch(t)
            expand(pool.at[xside, pl.ds(t & 1, 1)], [(ring(t), resident(_HOME2, t))], None, resident(_ALIAS2, t),
                   0, nsub - 1)

        return jax.lax.fori_loop(tab_ref[_CUTS, m], tab_ref[_CUTS, m + 1], phase2, carry)

    jax.lax.fori_loop(0, len(REDO) + 1, segment, 0)
    for t in (1, 0):
        for e in (0, 1):
            o_part(t, e).wait()


@jax.jit
def pallas_standalone__modern_conv_block_slak__vision_kernel(x, dw, w1, w2, grn_g, grn_b):
    B, H, W, C = x.shape
    c4 = 4 * C
    assert B == 1 and dw.shape == (1, 1, C) and C == 384 and w1.shape == (C, c4) and TM == c4
    nt = H * W // TM
    nsub = TM // (2 * R)
    nstr = 2 * nsub * (c4 // 128) - NRES
    assert nt * TM == H * W and nt % 2 == 0 and nsub % 3 == 0 and NRES >= 4 * (c4 // 128)
    table, nkept, nsent = _placement(nt, nstr)
    hbm = pl.BlockSpec(memory_space=pl.ANY)
    vmem = pl.BlockSpec(memory_space=pltpu.VMEM)
    out, _ = pl.pallas_call(
        functools.partial(_body, nt=nt),
        in_specs=[hbm, vmem, hbm, hbm, vmem, vmem, pl.BlockSpec(memory_space=pltpu.SMEM)],
        out_specs=[hbm, hbm],
        out_shape=[
            jax.ShapeDtypeStruct((nt, TM, C), x.dtype),
            jax.ShapeDtypeStruct((nsent, nstr, R // 2, 256), jnp.bfloat16),
        ],
        scratch_shapes=[
            pltpu.VMEM((2, 2, TM, C), x.dtype),
            pltpu.VMEM((nkept * NRES + NSTG * nstr, R // 2, 256), jnp.bfloat16),
            pltpu.VMEM((15, 4, 64, 128), jnp.uint32),
            pltpu.VMEM((15, 4, 64, 128), jnp.uint32),
            pltpu.VMEM((8, c4), jnp.float32),
            pltpu.VMEM((3, len(_PAIRS), R // 2, 256), jnp.uint32),
            pltpu.VMEM((4, 10, R, 128), jnp.float32),
            pltpu.VMEM((R // 16, 16, C), jnp.float32),
            pltpu.VMEM((8, C), jnp.float32),
            pltpu.SemaphoreType.DMA((NSTG,)),
            pltpu.SemaphoreType.DMA((2,)),
            pltpu.SemaphoreType.DMA((4,)),
            pltpu.SemaphoreType.DMA((4,)),
        ],
        compiler_params=pltpu.CompilerParams(vmem_limit_bytes=128 * 1024 * 1024),
    )(x.reshape(nt, TM, C), dw.reshape(1, C), w1, w2, grn_g, grn_b, table)
    return out.reshape(B, H, W, C)
```
